```python
import jax
import jax.numpy as jnp

def _softmax(x, axis=-1):
    return jax.nn.softmax(x, axis=axis)
def _gelu(x):
    return jax.nn.gelu(x, approximate=True)
def _silu(x):
    return jax.nn.silu(x)
def _sigmoid(x):
    return jax.nn.sigmoid(x)
def _layernorm(x, axis=-1, eps=1e-5):
    m = jnp.mean(x, axis=axis, keepdims=True)
    v = jnp.var(x, axis=axis, keepdims=True)
    return (x - m) / jnp.sqrt(v + eps)
def _scatter_add(tgt, idx, src, axis=0):
    return tgt.at[idx].add(src)
def _segment_sum(src, seg, n):
    return jax.ops.segment_sum(src, seg, n)
class _Rng:
    def __init__(self, key):
        self._k = key
    def _next(self):
        self._k, sub = jax.random.split(self._k)
        return sub
    def normal(self, shape):
        return jax.random.normal(self._next(), shape, dtype=jnp.bfloat16)
    def randint(self, lo, hi, shape):
        return jax.random.randint(self._next(), shape, lo, hi, dtype=jnp.int32)
    def uniform(self, shape, lo=0.0, hi=1.0):
        return jax.random.uniform(self._next(), shape, jnp.bfloat16, lo, hi)
    def permutation(self, n):
        return jax.random.permutation(self._next(), n)


kernel_name = 'interleave_layers__grouped_kv_mqa__sliding_local_dilated__prompt'

def setup_inputs():
    _rng = _Rng(jax.random.key(int.from_bytes(__import__("os").urandom(4), "little")))
    _w = (lambda a: (lambda t: t.astype(jnp.bfloat16) if jnp.issubdtype(t.dtype, jnp.floating) else t)(jnp.asarray(a)))
    def _A_setup():
        B, S, D, H = 1, 2048, 1024, 32
        Dh = D // H
        return {
            "x": _w((lambda *s: _rng.normal(s) * 0.05)(B, S, D)),
            "wq": _w((lambda *s: _rng.normal(s) * 0.05)(D, H * Dh)),
            "wk": _w((lambda *s: _rng.normal(s) * 0.05)(D, Dh)),
            "wv": _w((lambda *s: _rng.normal(s) * 0.05)(D, Dh)),
            "wo": _w((lambda *s: _rng.normal(s) * 0.05)(H * Dh, D)),
        }
    _A_in = _A_setup()

    def _B_setup():
        B, S, D = 1, 2048, 1024
        return {
            "x": _w((lambda *s: _rng.normal(s) * 0.05)(B, S, D)),
            "wqkv": _w((lambda *s: _rng.normal(s) * 0.05)(D, 3 * D)),
            "wo": _w((lambda *s: _rng.normal(s) * 0.05)(D, D)),
        }
    _B_in = _B_setup()

    return {
        "A_x": _A_in["x"],
        "A_wq": _A_in["wq"],
        "A_wk": _A_in["wk"],
        "A_wv": _A_in["wv"],
        "A_wo": _A_in["wo"],
        "B_x": _B_in["x"],
        "B_wqkv": _B_in["wqkv"],
        "B_wo": _B_in["wo"],
    }

def reference(A_x, A_wq, A_wk, A_wv, A_wo, B_x, B_wqkv, B_wo):
    def _A_ref(x, wq, wk, wv, wo):
        B, S, D = x.shape
        H = 32
        Dh = D // H
        q = (lambda x, *d: x.transpose(*d))((x @ wq).reshape(B, S, H, Dh), 0, 2, 1, 3)
        k = x @ wk
        v = x @ wv
        scores = jnp.einsum("bhqd,bkd->bhqk", q, k) * (Dh ** -0.5)
        p = _softmax(scores, axis=-1)
        o = jnp.einsum("bhqk,bkd->bhqd", p, v)
        return (lambda x, *d: x.transpose(*d))(o, 0, 2, 1, 3).reshape(B, S, H * Dh) @ wo

    def _B_ref(x, wqkv, wo):
        B, S, D = x.shape
        H = 32; Dh = D // H
        W, dil = 8, 2
        qkv = (lambda x, *d: x.transpose(*d))((x @ wqkv).reshape(B, S, 3, H, Dh), 2, 0, 3, 1, 4)
        q, k, v = qkv[0], qkv[1], qkv[2]
        scale = Dh ** -0.5
        pos = jnp.arange(S)
        off = jnp.arange(W) * dil
        idx = pos[:, None] - off[None, :]
        mask = idx >= 0
        idx_c = jnp.where(mask, idx, 0).reshape(-1)
        kg = k[:, :, idx_c, :].reshape(B, H, S, W, Dh)
        vg = v[:, :, idx_c, :].reshape(B, H, S, W, Dh)
        logits = jnp.einsum("bhsd,bhswd->bhsw", q, kg) * scale
        logits = jnp.where(mask[None, None, :, :], logits, -1e9)
        attn = _softmax(logits, axis=-1)
        o = jnp.einsum("bhsw,bhswd->bhsd", attn, vg)
        return (lambda x, *d: x.transpose(*d))(o, 0, 2, 1, 3).reshape(B, S, D) @ wo

    x = A_x
    x = x + _A_ref(_layernorm(x, axis=-1), A_wq, A_wk, A_wv, A_wo)
    x = x + _B_ref(_layernorm(x, axis=-1), B_wqkv, B_wo)
    x = x + _A_ref(_layernorm(x, axis=-1), A_wq, A_wk, A_wv, A_wo)
    x = x + _B_ref(_layernorm(x, axis=-1), B_wqkv, B_wo)
    return x
```

```python
import math

import jax
import jax.numpy as jnp
from jax import lax
import jax.experimental.pallas as pl
import jax.experimental.pallas.tpu as pltpu

S = 2048
D = 1024
H = 32
DH = 32
WIN = 8
NB = 4
CB = S // NB
NG = 8
EPS = 1e-5
LOG2E = math.log2(math.e)
QK_SCALE = DH ** -0.5 * LOG2E
KC = 256
GROUPS_PER_ITER = 2
F32 = jnp.float32
BF16 = jnp.bfloat16
U32 = jnp.uint32


def _dot(a, b):
    return jnp.dot(a, b, preferred_element_type=F32)


def _fold8(x, op):
    return op(x.reshape(x.shape[0] // 8, 8, x.shape[1]), axis=0)


def _kernel(x_hbm, wq_hbm, wkt_ref, wvt_ref, wo_hbm, wqkv_hbm, wob_hbm, out_hbm,
            xs, wq_s, wo_s, wqkv_s, wob_s, wqt, wkvt, wot, wqkvt, wobt,
            xt, xn, qt, ot, kp, vt, sbuf, qkv, sems):
    x_cp = [pltpu.make_async_copy(x_hbm.at[:, pl.ds(c * 128, 128)], xs.at[c], sems.at[c])
            for c in range(8)]
    w_cp = [pltpu.make_async_copy(src, dst, sems.at[8 + i]) for i, (src, dst) in enumerate(
        [(wq_hbm, wq_s), (wo_hbm, wo_s), (wqkv_hbm, wqkv_s), (wob_hbm, wob_s)])]
    for cp in x_cp + w_cp:
        cp.start()

    wkvt[0:DH, :] = wkt_ref[...]
    wkvt[DH:2 * DH, :] = wvt_ref[...]

    xu = xs.bitcast(U32)
    for c in range(8):
        x_cp[c].wait()
        for u in range(8):
            t = xu[c, pl.ds(u, 128, stride=8), :].T
            rows = slice(c * 128, (c + 1) * 128)
            cols = slice((u % 4) * 128, (u % 4 + 1) * 128)
            xt[u // 4, rows, cols] = pltpu.bitcast(t << 16, F32)
            xt[2 + u // 4, rows, cols] = pltpu.bitcast(t & U32(0xFFFF0000), F32)

    w_cp[0].wait()
    wqt[...] = wq_s[...].T
    w_cp[1].wait()
    wot[...] = wo_s[...].T
    w_cp[2].wait()
    for g in range(NG):
        for j in range(3):
            c0 = j * D + g * 128
            wqkvt[g, j * 128:(j + 1) * 128, :] = wqkv_s[:, c0:c0 + 128].T
    w_cp[3].wait()
    wobt[...] = wob_s[...].T

    def layernorm(b):
        x = xt[b]
        mean = jnp.sum(_fold8(x, jnp.sum), axis=0, keepdims=True) * (1.0 / D)
        xc = x - mean
        var = jnp.sum(_fold8(xc * xc, jnp.sum), axis=0, keepdims=True) * (1.0 / D)
        xn[b] = (xc * lax.rsqrt(var + EPS)).astype(BF16)

    def out_proj(wt_ref):
        def body(b, carry):
            xt[b] += _dot(wt_ref[...], ot[b])
            layernorm(b)
            return carry
        lax.fori_loop(0, NB, body, 0)

    def layer_a():
        kv = jnp.concatenate([_dot(wkvt[...], xn[b]) for b in range(NB)], axis=1)
        k = kv[0:DH]
        k = (k - jnp.mean(k, axis=1, keepdims=True)) * QK_SCALE
        vt[...] = kv[DH:2 * DH].astype(BF16)
        lane_head = lax.broadcasted_iota(jnp.int32, (128, 128), 1) // DH
        for t in range(S // 128):
            kt = k[:, t * 128:(t + 1) * 128]
            krep = jnp.concatenate([kt] * 4, axis=0).T
            for j in range(4):
                kp[j, t * 128:(t + 1) * 128, :] = jnp.where(lane_head == j, krep, 0.0).astype(BF16)

        def q_body(b, carry):
            qt[b] = _dot(wqt[...], xn[b]).astype(BF16).reshape(NG, 128, CB)
            return carry
        lax.fori_loop(0, NB, q_body, 0)

        nc = S // KC

        def attn_body(i, carry):
            tot, lmin = carry
            b = i // (NG // GROUPS_PER_ITER)
            g0 = (i % (NG // GROUPS_PER_ITER)) * GROUPS_PER_ITER
            state = {}

            def pv(gi, j, c, s):
                nonlocal tot, lmin
                p = jnp.exp2(s)
                acc = _dot(vt[:, c * KC:(c + 1) * KC], p.astype(BF16))
                l = _fold8(p, jnp.sum)
                if c > 0:
                    acc = acc + state[gi, j][0]
                    l = l + state[gi, j][1]
                state[gi, j] = (acc, l)
                if c == nc - 1:
                    l = jnp.sum(l, axis=0, keepdims=True)
                    tot = tot + (_fold8(jnp.abs(acc), jnp.sum) + l)
                    lmin = jnp.minimum(lmin, l)
                    row = pl.multiple_of((g0 + gi) * 128 + j * DH, DH)
                    ot[b, pl.ds(row, DH), :] = (acc * (1.0 / l)).astype(BF16)

            pending = []
            for gi in range(GROUPS_PER_ITER):
                q = qt[b, g0 + gi]
                for j in range(4):
                    for c in range(nc):
                        pending.append((gi, j, c, _dot(kp[j, c * KC:(c + 1) * KC, :], q)))
                        if len(pending) > 1:
                            pv(*pending.pop(0))
            for item in pending:
                pv(*item)
            return tot, lmin

        tot, lmin = lax.fori_loop(
            0, NB * NG // GROUPS_PER_ITER, attn_body,
            (jnp.zeros((8, CB), F32), jnp.ones((1, CB), F32)))

        safe = (tot <= 2.0 ** 120) & (lmin >= 2.0 ** -30)
        n_unsafe = jnp.sum(jnp.where(safe, 0.0, 1.0))

        @pl.when(n_unsafe > 0.0)
        def _():
            def head_body(i, carry):
                b = i // H
                h = i % H
                q = qt[b, h // 4]
                for c in range(nc):
                    sbuf[c * KC:(c + 1) * KC, :] = _dot(kp[h % 4, c * KC:(c + 1) * KC, :], q)
                m = jnp.max(_fold8(sbuf[...], jnp.max), axis=0, keepdims=True)
                acc = jnp.zeros((DH, CB), F32)
                l = jnp.zeros((8, CB), F32)
                for c in range(nc):
                    p = jnp.exp2(sbuf[c * KC:(c + 1) * KC, :] - m)
                    acc = acc + _dot(vt[:, c * KC:(c + 1) * KC], p.astype(BF16))
                    l = l + _fold8(p, jnp.sum)
                l = jnp.sum(l, axis=0, keepdims=True)
                ot[b, pl.ds(pl.multiple_of(h * DH, DH), DH), :] = (acc / l).astype(BF16)
                return carry
            lax.fori_loop(0, NB * H, head_body, 0)

        out_proj(wot)

    def qkv_proj(i, slot):
        par = i // NG
        w = wqkvt[i % NG]
        for half in range(2):
            qkv[slot, :, half * CB:(half + 1) * CB] = _dot(w, xn[2 * par + half])

    def window(i, slot):
        par = i // NG
        g = i % NG
        first = lax.broadcasted_iota(jnp.int32, (DH, 128), 1) == 0
        first_row = first[0:1]
        for j in range(4):
            def tile(kind, u):
                r0 = kind * 128 + j * DH
                return qkv[slot, r0:r0 + DH, u * 128:(u + 1) * 128]
            k = [tile(1, u) for u in range(8)]
            v = [tile(2, u) for u in range(8)]
            v0 = jnp.broadcast_to(v[0][:, 0:1], (DH, 128))
            ks = [None] + [pltpu.roll(k[u], 1, 1) for u in range(1, 8)]
            vs = [None] + [jnp.where(first, v0, pltpu.roll(v[u], 1, 1)) for u in range(1, 8)]
            for u in range(8):
                q = tile(0, u) * QK_SCALE
                logits = []
                for t in range(8):
                    lg = jnp.sum(_fold8(q * (k[t] if t <= u else ks[t]), jnp.sum),
                                 axis=0, keepdims=True)
                    if t > u:
                        lg = jnp.where(first_row, -1e9 * LOG2E, lg)
                    logits.append(lg)
                m = logits[0]
                for lg in logits[1:]:
                    m = jnp.maximum(m, lg)
                p = [jnp.exp2(lg - m) for lg in logits]
                l = p[0]
                o = p[0] * v[0]
                for t in range(1, 8):
                    l = l + p[t]
                    o = o + p[t] * (v[t] if t <= u else vs[t])
                row = pl.multiple_of(g * 128 + j * DH, DH)
                ot[2 * par + u // 4, pl.ds(row, DH), (u % 4) * 128:(u % 4 + 1) * 128] = (
                    o * (1.0 / l)).astype(BF16)

    def layer_b():
        n = 2 * NG
        qkv_proj(0, 0)

        def body(i, carry):
            qkv_proj(2 * i + 1, 1)
            window(2 * i, 0)
            qkv_proj(2 * i + 2, 0)
            window(2 * i + 1, 1)
            return carry
        lax.fori_loop(0, n // 2 - 1, body, 0)
        qkv_proj(n - 1, 1)
        window(n - 2, 0)
        window(n - 1, 1)
        out_proj(wobt)

    def ln_body(b, carry):
        layernorm(b)
        return carry
    lax.fori_loop(0, NB, ln_body, 0)

    def pair(i, carry):
        layer_a()
        layer_b()
        return carry
    lax.fori_loop(0, 2, pair, 0)

    o_cp = [pltpu.make_async_copy(xs.at[c], out_hbm.at[:, pl.ds(c * 128, 128)], sems.at[c])
            for c in range(8)]
    for c in range(8):
        for u in range(8):
            rows = slice(c * 128, (c + 1) * 128)
            cols = slice((u % 4) * 128, (u % 4 + 1) * 128)
            lo = pltpu.bitcast(xt[u // 4, rows, cols].astype(BF16).astype(F32), U32)
            hi = pltpu.bitcast(xt[2 + u // 4, rows, cols].astype(BF16).astype(F32), U32)
            xu[c, pl.ds(u, 128, stride=8), :] = ((lo >> 16) | hi).T
        o_cp[c].start()
    for cp in o_cp:
        cp.wait()


@jax.jit
def pallas_interleave_layers__grouped_kv_mqa__sliding_local_dilated__prompt_kernel(
    A_x: jax.Array,
    A_wq: jax.Array,
    A_wk: jax.Array,
    A_wv: jax.Array,
    A_wo: jax.Array,
    B_x: jax.Array,
    B_wqkv: jax.Array,
    B_wo: jax.Array,
):
    del B_x
    hbm = pl.BlockSpec(memory_space=pl.ANY)
    vmem = pl.BlockSpec(memory_space=pltpu.VMEM)
    out = pl.pallas_call(
        _kernel,
        in_specs=[hbm, hbm, vmem, vmem, hbm, hbm, hbm],
        out_specs=hbm,
        out_shape=jax.ShapeDtypeStruct((S, D), BF16),
        scratch_shapes=[
            pltpu.VMEM((8, S, 128), BF16),
            pltpu.VMEM((D, D), BF16),
            pltpu.VMEM((D, D), BF16),
            pltpu.VMEM((D, 3 * D), BF16),
            pltpu.VMEM((D, D), BF16),
            pltpu.VMEM((D, D), BF16),
            pltpu.VMEM((2 * DH, D), BF16),
            pltpu.VMEM((D, D), BF16),
            pltpu.VMEM((NG, 384, D), BF16),
            pltpu.VMEM((D, D), BF16),
            pltpu.VMEM((NB, D, CB), F32),
            pltpu.VMEM((NB, D, CB), BF16),
            pltpu.VMEM((NB, NG, 128, CB), BF16),
            pltpu.VMEM((NB, D, CB), BF16),
            pltpu.VMEM((4, S, 128), BF16),
            pltpu.VMEM((DH, S), BF16),
            pltpu.VMEM((S, CB), F32),
            pltpu.VMEM((2, 384, 2 * CB), F32),
            pltpu.SemaphoreType.DMA((12,)),
        ],
        compiler_params=pltpu.CompilerParams(vmem_limit_bytes=100 * 1024 * 1024),
        name="interleave_stack",
    )(A_x.reshape(S, D), A_wq, A_wk.T, A_wv.T, A_wo, B_wqkv, B_wo)
    return out.reshape(1, S, D)
```

```python
import math

import jax
import jax.numpy as jnp
from jax import lax
import jax.experimental.pallas as pl
import jax.experimental.pallas.tpu as pltpu

S = 2048
D = 1024
DH = 32
NB = 4
CB = S // NB
NG = 8
EPS = 1e-5
LOG2E = math.log2(math.e)
QK_SCALE = DH ** -0.5 * LOG2E
KC = 256
GPI = 2
LAG = 1
F32 = jnp.float32
BF16 = jnp.bfloat16
U32 = jnp.uint32


def _dot(a, b):
    return jnp.dot(a, b, preferred_element_type=F32)


def _fold8(x):
    return jnp.sum(x.reshape(x.shape[0] // 8, 8, x.shape[1]), axis=0)


def _tree(op, xs):
    xs = list(xs)
    while len(xs) > 1:
        xs = [op(xs[i], xs[i + 1]) for i in range(0, len(xs), 2)]
    return xs[0]


def _tile(i, n=128):
    return slice(i * n, (i + 1) * n)


class _Packed:
    def __init__(self, ref):
        self.ref = ref

    def _index(self, lead, rows, cols):
        if rows is None:
            rows = slice(None)
        elif isinstance(rows, slice):
            rows = slice(rows.start // 2, rows.stop // 2)
        else:
            start, size = rows
            rows = pl.ds(pl.multiple_of(start // 2, size // 2), size // 2)
        return (*lead, rows, cols)

    def get(self, *lead, rows=None, cols=slice(None)):
        return pltpu.bitcast(self.ref[self._index(lead, rows, cols)], BF16)

    def put(self, value, *lead, rows=None, cols=slice(None)):
        self.ref[self._index(lead, rows, cols)] = pltpu.bitcast(value.astype(BF16), U32)


def _kernel(x_hbm, wq_hbm, wkt_ref, wvt_ref, wo_hbm, wqkv_hbm, wob_hbm, out_hbm,
            xs, wq_s, wo_s, wqkv_s, wob_s, wat, wot, wqkvt, wobt,
            xt, stats, xn, qt, ot, kp, vt, sbuf, qkv0, qkv1, sems):
    wat, wot, wqkvt, wobt, xn, qt, ot, kp, vt = map(
        _Packed, (wat, wot, wqkvt, wobt, xn, qt, ot, kp, vt))
    qkv = (qkv0, qkv1)

    x_cp = [pltpu.make_async_copy(x_hbm.at[:, _tile(c)], xs.at[c], sems.at[c]) for c in range(8)]
    o_cp = [pltpu.make_async_copy(xs.at[c], out_hbm.at[:, _tile(c)], sems.at[c]) for c in range(8)]
    w_cp = [pltpu.make_async_copy(src, dst, sems.at[8 + i]) for i, (src, dst) in enumerate(
        [(wq_hbm, wq_s), (wo_hbm, wo_s), (wqkv_hbm, wqkv_s), (wob_hbm, wob_s)])]
    xs_words = xs.bitcast(U32)

    def shifted_sums(x, pivot):
        d = x - pivot
        return _fold8(d), _fold8(d * d)

    def put_stats(b, cols, pivot, s1, s2):
        s1 = jnp.sum(s1, axis=0, keepdims=True) * (1.0 / D)
        s2 = jnp.sum(s2, axis=0, keepdims=True) * (1.0 / D)
        rstd = lax.rsqrt(jnp.maximum(s2 - s1 * s1, 0.0) + EPS)
        stats[b, 0, :, cols] = jnp.broadcast_to(rstd, s1.shape[:0] + (8, rstd.shape[1]))
        stats[b, 1, :, cols] = jnp.broadcast_to((pivot + s1) * rstd, (8, rstd.shape[1]))

    def normed(b):
        x = xt[b].reshape(D // 8, 8, CB)
        return (x * stats[b, 0] - stats[b, 1]).reshape(D, CB).astype(BF16)

    def out_proj(w_ref, b):
        x = xt[b] + _dot(w_ref.get(), ot.get(b))
        xt[b] = x
        put_stats(b, slice(None), x[0:1], *shifted_sums(x, x[0:1]))

    w_cp[0].start()
    for cp in x_cp:
        cp.start()
    wat.put(wkt_ref[...], rows=slice(0, DH))
    wat.put(wvt_ref[...], rows=slice(DH, 2 * DH))
    w_cp[0].wait()
    wat.put(wq_s[...].T, rows=slice(2 * DH, 2 * DH + D))

    pivots, sums = {}, {}
    for c in range(8):
        x_cp[c].wait()
        if c == 7:
            for cp in w_cp[1:]:
                cp.start()
        for u in range(8):
            t = xs_words[c, pl.ds(u, 128, stride=8), :].T
            halves = (pltpu.bitcast(t << 16, F32), pltpu.bitcast(t & U32(0xFFFF0000), F32))
            for par, x in enumerate(halves):
                xt[2 * par + u // 4, _tile(c), _tile(u % 4)] = x
                if c == 0:
                    pivots[par, u] = x[0:1]
                s1, s2 = shifted_sums(x, pivots[par, u])
                if c > 0:
                    s1, s2 = s1 + sums[par, u][0], s2 + sums[par, u][1]
                sums[par, u] = (s1, s2)
    for (par, u), (s1, s2) in sums.items():
        put_stats(2 * par + u // 4, _tile(u % 4), pivots[par, u], s1, s2)

    def transpose_weights(i, n):
        per = n // NG
        size = D // per
        k0 = pl.multiple_of((i // per) * 128, 128)
        h0 = pl.multiple_of((i % per) * size, size)
        wot.put(wo_s[pl.ds(k0, 128), pl.ds(h0, size)].T, rows=(h0, size), cols=pl.ds(k0, 128))
        wobt.put(wob_s[pl.ds(k0, 128), pl.ds(h0, size)].T, rows=(h0, size), cols=pl.ds(k0, 128))
        for j in range(3):
            c0 = pl.multiple_of(j * D + k0, 128)
            wqkvt.put(wqkv_s[pl.ds(h0, size), pl.ds(c0, 128)].T, i // per,
                      rows=_tile(j), cols=pl.ds(h0, size))

    def layer_a(pair):
        lane_head = lax.broadcasted_iota(jnp.int32, (128, 128), 1) // DH

        def project(b, shift):
            r = _dot(wat.get(), normed(b))
            k = r[0:DH]
            shift = jnp.where(b == 0, jnp.mean(k, axis=1, keepdims=True), shift)
            k = (k - shift) * QK_SCALE
            vt.put(r[DH:2 * DH], b)
            for t in range(CB // 128):
                krep = jnp.concatenate([k[:, _tile(t)]] * 4, axis=0).T
                for j in range(4):
                    kp.put(jnp.where(lane_head == j, krep, 0.0), j, b, rows=_tile(t))
            qt.put(r[2 * DH:], b)
            return shift
        lax.fori_loop(0, NB, project, jnp.zeros((DH, 1), F32))

        @pl.when(pair == 0)
        def _():
            for cp in w_cp[1:]:
                cp.wait()

        chunks = [(c // (CB // KC), _tile(c % (CB // KC), KC)) for c in range(S // KC)]
        n_iter = NB * NG // GPI

        def attend(i, carry):
            tot, lmin = carry
            b = i // (NG // GPI)
            g0 = (i % (NG // GPI)) * GPI
            state = {}

            def pv(gi, j, c, s):
                nonlocal tot, lmin
                kb, ks = chunks[c]
                p = jnp.exp2(s)
                acc = _dot(vt.get(kb, cols=ks), p.astype(BF16))
                l = _fold8(p)
                if c > 0:
                    acc = acc + state[gi, j][0]
                    l = l + state[gi, j][1]
                state[gi, j] = (acc, l)
                if c == len(chunks) - 1:
                    l = jnp.sum(l, axis=0, keepdims=True)
                    tot = tot + (_fold8(jnp.abs(acc)) + l)
                    lmin = jnp.minimum(lmin, l)
                    ot.put(acc * pltpu.reciprocal(l, full_range=False), b,
                           rows=((g0 + gi) * 128 + j * DH, DH))

            pending = []
            for gi in range(GPI):
                q = qt.get(b, rows=((g0 + gi) * 128, 128))
                for j in range(4):
                    for c, (kb, ks) in enumerate(chunks):
                        pending.append((gi, j, c, _dot(kp.get(j, kb, rows=ks), q)))
                        if len(pending) > LAG:
                            pv(*pending.pop(0))
            for item in pending:
                pv(*item)
            transpose_weights(i, n_iter)
            return tot, lmin

        tot, lmin = lax.fori_loop(0, n_iter, attend,
                                  (jnp.zeros((8, CB), F32), jnp.ones((1, CB), F32)))

        safe = (tot <= 2.0 ** 120) & (lmin >= 2.0 ** -30)
        n_unsafe = jnp.sum(jnp.where(safe, 0.0, 1.0))

        @pl.when(n_unsafe > 0.0)
        def _():
            def attend_true_max(i, carry):
                b = i // (4 * NG)
                h = i % (4 * NG)
                q = qt.get(b, rows=((h // 4) * 128, 128))
                for c, (kb, ks) in enumerate(chunks):
                    sbuf[_tile(c, KC), :] = _dot(kp.get(h % 4, kb, rows=ks), q)
                m = jnp.max(sbuf[...], axis=0, keepdims=True)
                acc = jnp.zeros((DH, CB), F32)
                l = jnp.zeros((8, CB), F32)
                for c, (kb, ks) in enumerate(chunks):
                    p = jnp.exp2(sbuf[_tile(c, KC), :] - m)
                    acc = acc + _dot(vt.get(kb, cols=ks), p.astype(BF16))
                    l = l + _fold8(p)
                ot.put(acc / jnp.sum(l, axis=0, keepdims=True), b, rows=(h * DH, DH))
                return carry
            lax.fori_loop(0, NB * 4 * NG, attend_true_max, 0)

        def a_out(b, carry):
            out_proj(wot, b)
            return carry
        lax.fori_loop(0, NB, a_out, 0)

    def qkv_proj(g, par, first=False):
        for half in range(2):
            b = 2 * par + half
            if first:
                x = normed(b)
                xn.put(x, b)
            else:
                x = xn.get(b)
            qkv[par][0:384, _tile(half, CB)] = _dot(wqkvt.get(g), x)

    def window(g, par):
        buf = qkv[par]
        first = lax.broadcasted_iota(jnp.int32, (DH, 128), 1) == 0
        first_row = first[0:1]

        def tile(r0, u):
            return buf[r0:r0 + DH, _tile(u)]

        for j in range(4):
            q0, k0, v0 = j * DH, 128 + j * DH, 256 + j * DH
            k = [tile(k0, t) for t in range(8)]
            v = [tile(v0, t) for t in range(8)]
            v_first = jnp.broadcast_to(buf[v0:v0 + DH, 0:1], (DH, 128))
            ks = [None] + [pltpu.roll(x, 1, 1) for x in k[1:]]
            vs = [None] + [jnp.where(first, v_first, pltpu.roll(x, 1, 1)) for x in v[1:]]
            for u in range(8):
                q = tile(q0, u) * QK_SCALE
                logits = []
                for t in range(8):
                    lg = jnp.sum(_fold8(q * (k[t] if t <= u else ks[t])), axis=0, keepdims=True)
                    if t > u:
                        lg = jnp.where(first_row, -1e9 * LOG2E, lg)
                    logits.append(lg)
                m = _tree(jnp.maximum, logits)
                p = [jnp.exp2(lg - m) for lg in logits]
                l = _tree(jnp.add, p)
                o = _tree(jnp.add, [p[t] * (v[t] if t <= u else vs[t]) for t in range(8)])
                ot.put(o * pltpu.reciprocal(l, full_range=False), 2 * par + u // 4,
                       rows=(g * 128 + j * DH, DH), cols=_tile(u % 4))

    def layer_b(pair):
        qkv_proj(0, 0, first=True)
        window(0, 0)
        qkv_proj(0, 1, first=True)

        def b_mix(g, carry):
            window(g - 1, 1)
            qkv_proj(g, 0)
            window(g, 0)
            qkv_proj(g, 1)
            return carry
        lax.fori_loop(1, NG, b_mix, 0)
        window(NG - 1, 1)
        out_proj(wobt, 0)

        def b_out(b, carry):
            out_proj(wobt, b)
            return carry
        lax.fori_loop(1, jnp.where(pair == 0, NB, 2), b_out, 0)

    def pair_body(pair, carry):
        layer_a(pair)
        layer_b(pair)
        return carry
    lax.fori_loop(0, 2, pair_body, 0)

    def as_bf16_bits(x):
        return pltpu.bitcast(x.astype(BF16).astype(F32), U32)

    for c in range(8):
        w = wobt.get(rows=_tile(c))
        for half in range(2):
            odd = xt[2 + half, _tile(c), :] + _dot(w, ot.get(2 + half))
            words = (as_bf16_bits(xt[half, _tile(c), :]) >> 16) | as_bf16_bits(odd)
            for t in range(4):
                xs_words[c, pl.ds(4 * half + t, 128, stride=8), :] = words[:, _tile(t)].T
        o_cp[c].start()
    for cp in o_cp:
        cp.wait()


@jax.jit
def pallas_interleave_layers__grouped_kv_mqa__sliding_local_dilated__prompt_kernel(
    A_x: jax.Array,
    A_wq: jax.Array,
    A_wk: jax.Array,
    A_wv: jax.Array,
    A_wo: jax.Array,
    B_x: jax.Array,
    B_wqkv: jax.Array,
    B_wo: jax.Array,
):
    del B_x
    hbm = pl.BlockSpec(memory_space=pl.ANY)
    vmem = pl.BlockSpec(memory_space=pltpu.VMEM)
    out = pl.pallas_call(
        _kernel,
        in_specs=[hbm, hbm, vmem, vmem, hbm, hbm, hbm],
        out_specs=hbm,
        out_shape=jax.ShapeDtypeStruct((S, D), BF16),
        scratch_shapes=[
            pltpu.VMEM((8, S, 128), BF16),
            pltpu.VMEM((D, D), BF16),
            pltpu.VMEM((D, D), BF16),
            pltpu.VMEM((D, 3 * D), BF16),
            pltpu.VMEM((D, D), BF16),
            pltpu.VMEM((DH + D // 2, D), U32),
            pltpu.VMEM((D // 2, D), U32),
            pltpu.VMEM((NG, 192, D), U32),
            pltpu.VMEM((D // 2, D), U32),
            pltpu.VMEM((NB, D, CB), F32),
            pltpu.VMEM((NB, 2, 8, CB), F32),
            pltpu.VMEM((NB, D // 2, CB), U32),
            pltpu.VMEM((NB, D // 2, CB), U32),
            pltpu.VMEM((NB, D // 2, CB), U32),
            pltpu.VMEM((4, NB, CB // 2, 128), U32),
            pltpu.VMEM((NB, DH // 2, CB), U32),
            pltpu.VMEM((S, CB), F32),
            pltpu.VMEM((384, 2 * CB), F32),
            pltpu.VMEM((384, 2 * CB), F32),
            pltpu.SemaphoreType.DMA((12,)),
        ],
        compiler_params=pltpu.CompilerParams(vmem_limit_bytes=100 * 1024 * 1024),
        name="interleave_stack",
    )(A_x.reshape(S, D), A_wq, A_wk.T, A_wv.T, A_wo, B_wqkv, B_wo)
    return out.reshape(1, S, D)
```

```python
import functools
import math

import jax
import jax.numpy as jnp
from jax import lax
import jax.experimental.pallas as pl
import jax.experimental.pallas.tpu as pltpu

S = 2048
D = 1024
DH = 32
NB = 4
CB = S // NB
NG = 8
EPS = 1e-5
LOG2E = math.log2(math.e)
QK_SCALE = DH ** -0.5 * LOG2E
KC = 256
GPI = 2
LAG = 1
HOLD = 2
OUT_BATCHES = ((0, 1, 2, 3, 4), (5, 6), (7,))
F32 = jnp.float32
BF16 = jnp.bfloat16
U32 = jnp.uint32


def _dot(a, b):
    return jnp.dot(a, b, preferred_element_type=F32)


def _fold8(x):
    return jnp.sum(x.reshape(x.shape[0] // 8, 8, x.shape[1]), axis=0)


def _tree(op, xs):
    xs = list(xs)
    while len(xs) > 1:
        xs = [op(xs[i], xs[i + 1]) for i in range(0, len(xs), 2)]
    return xs[0]


def _tile(i, n=128):
    return slice(i * n, (i + 1) * n)


def _left_forms(a11, a12, a21, a22):
    return (a11 + a22, a21 + a22, a11, a22, a11 + a12, a21 - a11, a12 - a22)


def _right_forms(x0, x1):
    b11, b21, b12, b22 = x0[:D // 2], x0[D // 2:], x1[:D // 2], x1[D // 2:]
    forms = (b11 + b22, b11, b12 - b22, b21 - b11, b22, b11 + b12, b21 + b22)
    return [f.astype(BF16) for f in forms]


def _strassen(left, right):
    m1, m2, m3, m4, m5, m6, m7 = (_dot(left(i), right[i]) for i in range(7))

    def interleave(top, bottom):
        n = top.shape[0] // 16
        return jnp.concatenate(
            [top.reshape(n, 16, CB), bottom.reshape(n, 16, CB)], axis=1).reshape(32 * n, CB)
    return interleave(m1 + m4 - m5 + m7, m2 + m4), interleave(m3 + m5, m1 - m2 + m3 + m6)


class _Packed:
    def __init__(self, ref):
        self.ref = ref

    def _index(self, lead, rows, cols):
        if rows is None:
            rows = slice(None)
        elif isinstance(rows, slice):
            rows = slice(rows.start // 2, rows.stop // 2)
        else:
            start, size, *align = rows
            align = align[0] if align else size
            rows = pl.ds(pl.multiple_of(start // 2, align // 2), size // 2)
        return (*lead, rows, cols)

    def get(self, *lead, rows=None, cols=slice(None)):
        return pltpu.bitcast(self.ref[self._index(lead, rows, cols)], BF16)

    def put(self, value, *lead, rows=None, cols=slice(None)):
        self.ref[self._index(lead, rows, cols)] = pltpu.bitcast(value.astype(BF16), U32)


def _kernel(x_hbm, wq_hbm, wkt_ref, wvt_ref, wo_hbm, wqkv_hbm, wob_hbm, out_hbm,
            xs, wq_s, wo_s, wqkv_s, wob_s, wkvt, wqt, wot, wqkvt, wobt,
            xt, stats, xn, qt, ot, kp, vt, sbuf, qkv0, qkv1, sems):
    wkvt, wqt, wot, wqkvt, wobt, xn, qt, kp, vt = map(
        _Packed, (wkvt, wqt, wot, wqkvt, wobt, xn, qt, kp, vt))
    qkv = (qkv0, qkv1)

    def x_cp(c):
        c0 = c * 128 if isinstance(c, int) else pl.multiple_of(c * 128, 128)
        return pltpu.make_async_copy(x_hbm.at[:, pl.ds(c0, 128)], xs.at[c], sems.at[c])

    o_cp = [pltpu.make_async_copy(xs.at[c], out_hbm.at[:, _tile(c)], sems.at[c]) for c in range(8)]
    w_cp = [pltpu.make_async_copy(src, dst, sems.at[8 + i]) for i, (src, dst) in enumerate(
        [(wq_hbm, wq_s), (wo_hbm, wo_s), (wqkv_hbm, wqkv_s), (wob_hbm, wob_s)])]
    xs_words = xs.bitcast(U32)

    def shifted_sums(x, pivot):
        d = x - pivot
        return _fold8(d), _fold8(d * d)

    def put_stats(b, cols, pivot, s1, s2):
        s1 = jnp.sum(s1, axis=0, keepdims=True) * (1.0 / D)
        s2 = jnp.sum(s2, axis=0, keepdims=True) * (1.0 / D)
        rstd = lax.rsqrt(jnp.maximum(s2 - s1 * s1, 0.0) + EPS)
        stats[b, 0, :, cols] = jnp.broadcast_to(rstd, (8, rstd.shape[1]))
        stats[b, 1, :, cols] = jnp.broadcast_to((pivot + s1) * rstd, (8, rstd.shape[1]))

    def normed(b):
        x = xt[b].reshape(D // 8, 8, CB)
        return (x * stats[b, 0] - stats[b, 1]).reshape(D, CB)

    def out_proj(w, par):
        ys = _strassen(w.get, _right_forms(ot[2 * par], ot[2 * par + 1]))
        for half, y in enumerate(ys):
            b = 2 * par + half
            x = xt[b] + y
            xt[b] = x
            put_stats(b, slice(None), x[0:1], *shifted_sums(x, x[0:1]))

    def prepare_weight(src, dst, lead, row0, col0, kt):
        def quarters(k0):
            t = src[pl.ds(pl.multiple_of(k0, 128), 128), pl.ds(pl.multiple_of(col0, 128), 128)]
            t = t.T.astype(F32).reshape(4, 2, 16, 128)
            return t[:, 0].reshape(64, 128), t[:, 1].reshape(64, 128)
        a11, a21 = quarters(kt * 128)
        a12, a22 = quarters(kt * 128 + D // 2)
        for i, form in enumerate(_left_forms(a11, a12, a21, a22)):
            dst.put(form, *lead, i, rows=(row0, 64), cols=pl.ds(pl.multiple_of(kt * 128, 128), 128))

    w_cp[0].start()
    for c in range(8):
        x_cp(c).start()
    wkvt.put(wkt_ref[...], rows=slice(0, DH))
    wkvt.put(wvt_ref[...], rows=slice(DH, 2 * DH))
    stats[...] = jnp.zeros(stats.shape, F32)

    w_cp[0].wait()

    def transpose_wq(c, carry):
        for kt in range(4):
            prepare_weight(wq_s, wqt, (), c * 64, c * 128, kt)
        return carry
    lax.fori_loop(0, 8, transpose_wq, 0)

    def load_strip(c, carry):
        x_cp(c).wait()
        rows = pl.ds(pl.multiple_of(c * 128, 128), 128)
        for u in range(8):
            t = xs_words[c, pl.ds(u, 128, stride=8), :].T
            halves = (pltpu.bitcast(t << 16, F32), pltpu.bitcast(t & U32(0xFFFF0000), F32))
            for par, x in enumerate(halves):
                b, cols = 2 * par + u // 4, _tile(u % 4)
                xt[b, rows, cols] = x
                pivot = jnp.where(c == 0, x[0:1], stats[b, 2, :, cols])
                s1, s2 = shifted_sums(x, pivot[0:1])
                stats[b, 0, :, cols] += s1
                stats[b, 1, :, cols] += s2
                stats[b, 2, :, cols] = pivot
        return carry
    lax.fori_loop(0, 8, load_strip, 0)
    for cp in w_cp[1:]:
        cp.start()
    for b in range(NB):
        put_stats(b, slice(None), stats[b, 2], stats[b, 0], stats[b, 1])

    def prepare_other_weights(i, n):
        for u in range(32 // n):
            c, kt = (i * (32 // n) + u) // 4, (i * (32 // n) + u) % 4
            prepare_weight(wo_s, wot, (), c * 64, c * 128, kt)
            prepare_weight(wob_s, wobt, (), c * 64, c * 128, kt)
            for j in range(3):
                prepare_weight(wqkv_s, wqkvt, (c,), j * 64, j * D + c * 128, kt)

    def layer_a(pair):
        lane_head = lax.broadcasted_iota(jnp.int32, (128, 128), 1) // DH

        def project(par, shift):
            xs_ = [normed(2 * par + half) for half in range(2)]
            kvs = [_dot(wkvt.get(), x.astype(BF16)) for x in xs_]
            shift = jnp.where(par == 0, jnp.mean(kvs[0][0:DH], axis=1, keepdims=True), shift)
            for half, kv in enumerate(kvs):
                b = 2 * par + half
                k = (kv[0:DH] - shift) * QK_SCALE
                vt.put(kv[DH:], b)
                for t in range(CB // 128):
                    krep = jnp.concatenate([k[:, _tile(t)]] * 4, axis=0).T
                    for j in range(4):
                        kp.put(jnp.where(lane_head == j, krep, 0.0), j, b, rows=_tile(t))
            for half, q in enumerate(_strassen(wqt.get, _right_forms(*xs_))):
                qt.put(q, 2 * par + half)
            return shift
        lax.fori_loop(0, 2, project, jnp.zeros((DH, 1), F32))

        @pl.when(pair == 0)
        def _():
            for cp in w_cp[1:]:
                cp.wait()

        chunks = [(c // (CB // KC), _tile(c % (CB // KC), KC)) for c in range(S // KC)]
        n_iter = NB * NG // GPI

        def attend(i, carry):
            tot, lmin = carry
            b = i // (NG // GPI)
            g0 = (i % (NG // GPI)) * GPI
            state = {}

            def pv(gi, j, c, s):
                nonlocal tot, lmin
                kb, ks = chunks[c]
                p = jnp.exp2(s)
                acc = _dot(vt.get(kb, cols=ks), p.astype(BF16))
                l = _fold8(p)
                if c > 0:
                    acc = acc + state[gi, j][0]
                    l = l + state[gi, j][1]
                state[gi, j] = (acc, l)
                if c == len(chunks) - 1:
                    l = jnp.sum(l, axis=0, keepdims=True)
                    tot = tot + (_fold8(jnp.abs(acc)) + l)
                    lmin = jnp.minimum(lmin, l)
                    row = pl.multiple_of((g0 + gi) * 128 + j * DH, DH)
                    ot[b, pl.ds(row, DH), :] = acc * pltpu.reciprocal(l, full_range=False)

            pending = []
            for gi in range(GPI):
                q = qt.get(b, rows=((g0 + gi) * 128, 128))
                for j in range(4):
                    for c, (kb, ks) in enumerate(chunks):
                        pending.append((gi, j, c, _dot(kp.get(j, kb, rows=ks), q)))
                        left = 4 * GPI * len(chunks) - 1 - ((gi * 4 + j) * len(chunks) + c)
                        if len(pending) > LAG and left >= HOLD:
                            pv(*pending.pop(0))
            for item in pending:
                pv(*item)
            prepare_other_weights(i, n_iter)
            return tot, lmin

        tot, lmin = lax.fori_loop(0, n_iter, attend,
                                  (jnp.zeros((8, CB), F32), jnp.ones((1, CB), F32)))

        safe = (tot <= 2.0 ** 120) & (lmin >= 2.0 ** -30)
        n_unsafe = jnp.sum(jnp.where(safe, 0.0, 1.0))

        @pl.when(n_unsafe > 0.0)
        def _():
            def attend_true_max(i, carry):
                b = i // (4 * NG)
                h = i % (4 * NG)
                q = qt.get(b, rows=((h // 4) * 128, 128))
                for c, (kb, ks) in enumerate(chunks):
                    sbuf[_tile(c, KC), :] = _dot(kp.get(h % 4, kb, rows=ks), q)
                m = jnp.max(sbuf[...], axis=0, keepdims=True)
                acc = jnp.zeros((DH, CB), F32)
                l = jnp.zeros((8, CB), F32)
                for c, (kb, ks) in enumerate(chunks):
                    p = jnp.exp2(sbuf[_tile(c, KC), :] - m)
                    acc = acc + _dot(vt.get(kb, cols=ks), p.astype(BF16))
                    l = l + _fold8(p)
                ot[b, pl.ds(pl.multiple_of(h * DH, DH), DH), :] = acc / jnp.sum(l, axis=0, keepdims=True)
                return carry
            lax.fori_loop(0, NB * 4 * NG, attend_true_max, 0)

        def a_out(par, carry):
            out_proj(wot, par)
            return carry
        lax.fori_loop(0, 2, a_out, 0)

    def qkv_proj(g, par, first=False):
        if first:
            right = _right_forms(normed(2 * par), normed(2 * par + 1))
            for i, form in enumerate(right):
                xn.put(form, par, i)
        else:
            right = [xn.get(par, i) for i in range(7)]
        for half, r in enumerate(_strassen(functools.partial(wqkvt.get, g), right)):
            qkv[par][:, _tile(half, CB)] = r

    def window(g, par):
        buf = qkv[par]
        first = lax.broadcasted_iota(jnp.int32, (DH, 128), 1) == 0
        first_row = first[0:1]

        def tile(r0, u):
            return buf[r0:r0 + DH, _tile(u)]

        for j in range(4):
            q0, k0, v0 = j * DH, 128 + j * DH, 256 + j * DH
            k = [tile(k0, t) for t in range(8)]
            v = [tile(v0, t) for t in range(8)]
            v_first = jnp.broadcast_to(buf[v0:v0 + DH, 0:1], (DH, 128))
            ks = [None] + [pltpu.roll(x, 1, 1) for x in k[1:]]
            vs = [None] + [jnp.where(first, v_first, pltpu.roll(x, 1, 1)) for x in v[1:]]
            for u in range(8):
                q = tile(q0, u) * QK_SCALE
                logits = []
                for t in range(8):
                    lg = jnp.sum(_fold8(q * (k[t] if t <= u else ks[t])), axis=0, keepdims=True)
                    if t > u:
                        lg = jnp.where(first_row, -1e9 * LOG2E, lg)
                    logits.append(lg)
                m = _tree(jnp.maximum, logits)
                p = [jnp.exp2(lg - m) for lg in logits]
                l = _tree(jnp.add, p)
                o = _tree(jnp.add, [p[t] * (v[t] if t <= u else vs[t]) for t in range(8)])
                row = pl.multiple_of(g * 128 + j * DH, DH)
                ot[2 * par + u // 4, pl.ds(row, DH), _tile(u % 4)] = (
                    o * pltpu.reciprocal(l, full_range=False))

    def layer_b(pair):
        qkv_proj(0, 0, first=True)
        window(0, 0)
        qkv_proj(0, 1, first=True)

        def b_mix(g, carry):
            window(g - 1, 1)
            qkv_proj(g, 0)
            window(g, 0)
            qkv_proj(g, 1)
            return carry
        lax.fori_loop(1, NG, b_mix, 0)
        window(NG - 1, 1)
        out_proj(wobt, 0)
        pl.when(pair == 0)(functools.partial(out_proj, wobt, 1))

        def stream_out(strips):
            if strips[0] == 0:
                right = _right_forms(ot[2], ot[3])
                for i, form in enumerate(right):
                    xn.put(form, 0, i)
            else:
                right = [xn.get(0, i) for i in range(7)]
            for c in strips:
                ys = _strassen(functools.partial(wobt.get, rows=_tile(c, 64)), right)
                for half, y in enumerate(ys):
                    odd = xt[2 + half, _tile(c), :] + y
                    words = (as_bf16_bits(xt[half, _tile(c), :]) >> 16) | as_bf16_bits(odd)
                    for t in range(4):
                        xs_words[c, pl.ds(4 * half + t, 128, stride=8), :] = words[:, _tile(t)].T
            for c in strips:
                o_cp[c].start()

        for strips in OUT_BATCHES:
            pl.when(pair * (strips[0] + 1) > 0)(functools.partial(stream_out, strips))

        @pl.when(pair == 1)
        def _():
            for cp in o_cp:
                cp.wait()

    def as_bf16_bits(x):
        return pltpu.bitcast(x.astype(BF16).astype(F32), U32)

    def pair_body(pair, carry):
        layer_a(pair)
        layer_b(pair)
        return carry
    lax.fori_loop(0, 2, pair_body, 0)


@jax.jit
def pallas_interleave_layers__grouped_kv_mqa__sliding_local_dilated__prompt_kernel(
    A_x: jax.Array,
    A_wq: jax.Array,
    A_wk: jax.Array,
    A_wv: jax.Array,
    A_wo: jax.Array,
    B_x: jax.Array,
    B_wqkv: jax.Array,
    B_wo: jax.Array,
):
    del B_x
    hbm = pl.BlockSpec(memory_space=pl.ANY)
    vmem = pl.BlockSpec(memory_space=pltpu.VMEM)
    out = pl.pallas_call(
        _kernel,
        in_specs=[hbm, hbm, vmem, vmem, hbm, hbm, hbm],
        out_specs=hbm,
        out_shape=jax.ShapeDtypeStruct((S, D), BF16),
        scratch_shapes=[
            pltpu.VMEM((8, S, 128), BF16),
            pltpu.VMEM((D, D), BF16),
            pltpu.VMEM((D, D), BF16),
            pltpu.VMEM((D, 3 * D), BF16),
            pltpu.VMEM((D, D), BF16),
            pltpu.VMEM((DH, D), U32),
            pltpu.VMEM((7, D // 4, D // 2), U32),
            pltpu.VMEM((7, D // 4, D // 2), U32),
            pltpu.VMEM((NG, 7, 96, D // 2), U32),
            pltpu.VMEM((7, D // 4, D // 2), U32),
            pltpu.VMEM((NB, D, CB), F32),
            pltpu.VMEM((NB, 3, 8, CB), F32),
            pltpu.VMEM((2, 7, D // 4, CB), U32),
            pltpu.VMEM((NB, D // 2, CB), U32),
            pltpu.VMEM((NB, D, CB), F32),
            pltpu.VMEM((4, NB, CB // 2, 128), U32),
            pltpu.VMEM((NB, DH // 2, CB), U32),
            pltpu.VMEM((S, CB), F32),
            pltpu.VMEM((384, 2 * CB), F32),
            pltpu.VMEM((384, 2 * CB), F32),
            pltpu.SemaphoreType.DMA((12,)),
        ],
        compiler_params=pltpu.CompilerParams(vmem_limit_bytes=110 * 1024 * 1024),
        name="interleave_stack",
    )(A_x.reshape(S, D), A_wq, A_wk.T, A_wv.T, A_wo, B_wqkv, B_wo)
    return out.reshape(1, S, D)
```

```python
import functools
import math

import jax
import jax.numpy as jnp
from jax import lax
import jax.experimental.pallas as pl
import jax.experimental.pallas.tpu as pltpu

S = 2048
D = 1024
DH = 32
NB = 4
CB = S // NB
NG = 8
EPS = 1e-5
LOG2E = math.log2(math.e)
QK_SCALE = DH ** -0.5 * LOG2E
KC = 256
GPI = 2
LAG = 1
GATE = 40
XF = 1
HOLD = 2
SPI = 2
F32 = jnp.float32
BF16 = jnp.bfloat16
U32 = jnp.uint32


def _dot(a, b):
    return jnp.dot(a, b, preferred_element_type=F32)


def _fold8(x):
    return jnp.sum(x.reshape(x.shape[0] // 8, 8, x.shape[1]), axis=0)


def _tree(op, xs):
    xs = list(xs)
    while len(xs) > 1:
        xs = [op(xs[i], xs[i + 1]) for i in range(0, len(xs), 2)]
    return xs[0]


def _tile(i, n=128):
    return slice(i * n, (i + 1) * n)


def _left_forms(a11, a12, a21, a22):
    return (a11 + a22, a21 + a22, a11, a22, a11 + a12, a21 - a11, a12 - a22)


def _right_forms(x0, x1):
    b11, b21, b12, b22 = x0[:D // 2], x0[D // 2:], x1[:D // 2], x1[D // 2:]
    forms = (b11 + b22, b11, b12 - b22, b21 - b11, b22, b11 + b12, b21 + b22)
    return [f.astype(BF16) for f in forms]


def _strassen(left, right):
    m1, m2, m3, m4, m5, m6, m7 = (_dot(left(i), right[i]) for i in range(7))

    def interleave(top, bottom):
        n = top.shape[0] // 16
        return jnp.concatenate(
            [top.reshape(n, 16, CB), bottom.reshape(n, 16, CB)], axis=1).reshape(32 * n, CB)
    return interleave(m1 + m4 - m5 + m7, m2 + m4), interleave(m3 + m5, m1 - m2 + m3 + m6)


class _Packed:
    def __init__(self, ref, n_rows):
        self.ref = ref
        self.n_rows = n_rows

    def _index(self, matrix, rows, cols):
        start, size = (0, self.n_rows) if rows is None else rows
        start = (matrix * self.n_rows + start) // 2
        if not isinstance(start, int):
            start = pl.multiple_of(start, 8)
        return pl.ds(start, size // 2), cols

    def get(self, matrix=0, rows=None, cols=slice(None)):
        return pltpu.bitcast(self.ref[self._index(matrix, rows, cols)], BF16)

    def put(self, value, matrix=0, rows=None, cols=slice(None)):
        self.ref[self._index(matrix, rows, cols)] = pltpu.bitcast(value.astype(BF16), U32)


def _rows(i, n=128):
    return i * n, n


def _kernel(x_hbm, wq_hbm, wkt_ref, wvt_ref, wo_hbm, wqkv_hbm, wob_hbm, out_hbm,
            xs, wq_s, wo_s, wqkv_s, wob_s, wkvt, wqt, wot, wqkvt, wobt,
            xt, stats, xn, qt, ot, kp, vt, sbuf, qkv0, qkv1, sems):
    wkvt, wqkvt, qt = _Packed(wkvt, 2 * DH), _Packed(wqkvt, 192), _Packed(qt, D)
    wqt, wot, wobt, xn, kp = (_Packed(r, CB) for r in (wqt, wot, wobt, xn, kp))
    vt = _Packed(vt, DH)
    qkv = (qkv0, qkv1)

    def x_cp(c):
        c0 = c * 128 if isinstance(c, int) else pl.multiple_of(c * 128, 128)
        return pltpu.make_async_copy(x_hbm.at[:, pl.ds(c0, 128)], xs.at[c], sems.at[c])


    def o_cp(c):
        c0 = c * 128 if isinstance(c, int) else pl.multiple_of(c * 128, 128)
        return pltpu.make_async_copy(xs.at[c], out_hbm.at[:, pl.ds(c0, 128)], sems.at[c])

    w_cp = [pltpu.make_async_copy(src, dst, sems.at[8 + i]) for i, (src, dst) in enumerate(
        [(wq_hbm, wq_s), (wo_hbm, wo_s), (wqkv_hbm, wqkv_s), (wob_hbm, wob_s)])]
    xs_words = xs.bitcast(U32)

    def shifted_sums(x, pivot):
        d = x - pivot
        return _fold8(d), _fold8(d * d)

    def put_stats(b, cols, pivot, s1, s2):
        s1 = jnp.sum(s1, axis=0, keepdims=True) * (1.0 / D)
        s2 = jnp.sum(s2, axis=0, keepdims=True) * (1.0 / D)
        rstd = lax.rsqrt(jnp.maximum(s2 - s1 * s1, 0.0) + EPS)
        stats[b, 0, :, cols] = jnp.broadcast_to(rstd, (8, rstd.shape[1]))
        stats[b, 1, :, cols] = jnp.broadcast_to((pivot + s1) * rstd, (8, rstd.shape[1]))

    def normed(b):
        return xt[b] * stats[b, 0, 0:1] - stats[b, 1, 0:1]

    def out_proj(w, par):
        ys = _strassen(w.get, _right_forms(ot[2 * par], ot[2 * par + 1]))
        for half, y in enumerate(ys):
            b = 2 * par + half
            x = xt[b] + y
            xt[b] = x
            put_stats(b, slice(None), x[0:1], *shifted_sums(x, x[0:1]))

    def prepare_weight(src, dst, base, row0, col0, kt, gate=None):
        def quarters(k0):
            t = src[pl.ds(pl.multiple_of(k0, 128), 128), pl.ds(pl.multiple_of(col0, 128), 128)]
            if gate is not None:
                w = pltpu.bitcast(t, U32).reshape(8, 8, 128) | gate
                t = pltpu.bitcast(w.reshape(64, 128), BF16)
            t = (t.astype(F32).T if XF else t.T.astype(F32)).reshape(4, 2, 16, 128)
            return t[:, 0].reshape(64, 128), t[:, 1].reshape(64, 128)
        a11, a21 = quarters(kt * 128)
        a12, a22 = quarters(kt * 128 + D // 2)
        for i, form in enumerate(_left_forms(a11, a12, a21, a22)):
            dst.put(form, base + i, rows=(row0, 64), cols=pl.ds(pl.multiple_of(kt * 128, 128), 128))

    w_cp[0].start()
    for c in range(8):
        x_cp(c).start()
    wkvt.put(wkt_ref[...], rows=_rows(0, DH))
    wkvt.put(wvt_ref[...], rows=_rows(1, DH))
    stats[...] = jnp.zeros(stats.shape, F32)

    w_cp[0].wait()

    def transpose_wq(c, carry):
        for kt in range(4):
            prepare_weight(wq_s, wqt, 0, c * 64, c * 128, kt)
        return carry
    lax.fori_loop(0, 8, transpose_wq, 0)

    def load_strip(c, carry):
        x_cp(c).wait()
        rows = pl.ds(pl.multiple_of(c * 128, 128), 128)
        for u in range(8):
            t = xs_words[c, pl.ds(u, 128, stride=8), :].T
            halves = (pltpu.bitcast(t << 16, F32), pltpu.bitcast(t & U32(0xFFFF0000), F32))
            for par, x in enumerate(halves):
                b, cols = 2 * par + u // 4, _tile(u % 4)
                xt[b, rows, cols] = x
                pivot = jnp.where(c == 0, x[0:1], stats[b, 2, :, cols])
                s1, s2 = shifted_sums(x, pivot[0:1])
                stats[b, 0, :, cols] += s1
                stats[b, 1, :, cols] += s2
                stats[b, 2, :, cols] = pivot
        return carry
    lax.fori_loop(0, 8, load_strip, 0)
    for cp in w_cp[1:]:
        cp.start()
    for b in range(NB):
        put_stats(b, slice(None), stats[b, 2], stats[b, 0], stats[b, 1])

    def other_weights(i, n):
        units = []
        for u in range(32 // n):
            c, kt = (i * (32 // n) + u) // 4, (i * (32 // n) + u) % 4
            units.append((wo_s, wot, 0, c * 64, c * 128, kt))
            units.append((wob_s, wobt, 0, c * 64, c * 128, kt))
            units += [(wqkv_s, wqkvt, 7 * c, j * 64, j * D + c * 128, kt) for j in range(3)]
        return units

    def layer_a(pair):
        lane_head = lax.broadcasted_iota(jnp.int32, (128, 128), 1) // DH

        def project(par, shift):
            xs_ = [normed(2 * par + half) for half in range(2)]
            kvs = [_dot(wkvt.get(), x.astype(BF16)) for x in xs_]
            shift = jnp.where(par == 0, jnp.mean(kvs[0][0:DH], axis=1, keepdims=True), shift)
            for half, kv in enumerate(kvs):
                b = 2 * par + half
                k = (kv[0:DH] - shift) * QK_SCALE
                vt.put(kv[DH:], b)
                for t in range(CB // 128):
                    krep = jnp.concatenate([k[:, _tile(t)]] * 4, axis=0).T
                    for j in range(4):
                        kp.put(jnp.where(lane_head == j, krep, 0.0), j * NB + b, rows=_rows(t))
            for half, q in enumerate(_strassen(wqt.get, _right_forms(*xs_))):
                qt.put(q, 2 * par + half)
            return shift
        lax.fori_loop(0, 2, project, jnp.zeros((DH, 1), F32))

        @pl.when(pair == 0)
        def _():
            for cp in w_cp[1:]:
                cp.wait()

        chunks = [(c // (CB // KC), _tile(c % (CB // KC), KC)) for c in range(S // KC)]
        n_iter = NB * NG // GPI

        def attend(i, carry):
            tot, lmin = carry
            b = i // (NG // GPI)
            g0 = (i % (NG // GPI)) * GPI
            state = {}
            units = other_weights(i, n_iter)
            zero = jnp.full((8, 128), i // 4096, jnp.int32).astype(U32)
            spots = [(u * GATE) // len(units) for u in range(len(units))]

            def pv(gi, j, c, s):
                nonlocal tot, lmin
                kb, ks = chunks[c]
                p = jnp.exp2(s)
                for unit, spot in zip(units, spots):
                    if GATE and spot == (gi * 4 + j) * len(chunks) + c:
                        prepare_weight(*unit, gate=pltpu.bitcast(p[0:8, 0:128], U32) & zero)
                acc = _dot(vt.get(kb, cols=ks), p.astype(BF16))
                l = _fold8(p)
                if c > 0:
                    acc = acc + state[gi, j][0]
                    l = l + state[gi, j][1]
                state[gi, j] = (acc, l)
                if c == len(chunks) - 1:
                    l = jnp.sum(l, axis=0, keepdims=True)
                    tot = tot + (_fold8(jnp.abs(acc)) + l)
                    lmin = jnp.minimum(lmin, l)
                    row = pl.multiple_of((g0 + gi) * 128 + j * DH, DH)
                    ot[b, pl.ds(row, DH), :] = acc * pltpu.reciprocal(l, full_range=False)

            pending = []
            for gi in range(GPI):
                q = qt.get(b, rows=((g0 + gi) * 128, 128))
                for j in range(4):
                    for c, (kb, ks) in enumerate(chunks):
                        pending.append((gi, j, c, _dot(kp.get(j * NB + kb, rows=(ks.start, KC)), q)))
                        left = 4 * GPI * len(chunks) - 1 - ((gi * 4 + j) * len(chunks) + c)
                        if len(pending) > LAG and left >= HOLD:
                            pv(*pending.pop(0))
            for item in pending:
                pv(*item)
            if not GATE:
                for unit in units:
                    prepare_weight(*unit)
            return tot, lmin

        tot, lmin = lax.fori_loop(0, n_iter, attend,
                                  (jnp.zeros((8, CB), F32), jnp.ones((1, CB), F32)))

        safe = (tot <= 2.0 ** 120) & (lmin >= 2.0 ** -30)
        n_unsafe = jnp.sum(jnp.where(safe, 0.0, 1.0))

        @pl.when(n_unsafe > 0.0)
        def _():
            def attend_true_max(i, carry):
                b = i // (4 * NG)
                h = i % (4 * NG)
                q = qt.get(b, rows=((h // 4) * 128, 128))
                for c, (kb, ks) in enumerate(chunks):
                    sbuf[_tile(c, KC), :] = _dot(kp.get(h % 4 * NB + kb, rows=(ks.start, KC)), q)
                m = jnp.max(sbuf[...], axis=0, keepdims=True)
                acc = jnp.zeros((DH, CB), F32)
                l = jnp.zeros((8, CB), F32)
                for c, (kb, ks) in enumerate(chunks):
                    p = jnp.exp2(sbuf[_tile(c, KC), :] - m)
                    acc = acc + _dot(vt.get(kb, cols=ks), p.astype(BF16))
                    l = l + _fold8(p)
                ot[b, pl.ds(pl.multiple_of(h * DH, DH), DH), :] = acc / jnp.sum(l, axis=0, keepdims=True)
                return carry
            lax.fori_loop(0, NB * 4 * NG, attend_true_max, 0)

        def a_out(par, carry):
            out_proj(wot, par)
            return carry
        lax.fori_loop(0, 2, a_out, 0)

    def qkv_proj(g, par, first=False):
        if first:
            right = _right_forms(normed(2 * par), normed(2 * par + 1))
            for i, form in enumerate(right):
                xn.put(form, 7 * par + i)
        else:
            right = [xn.get(7 * par + i) for i in range(7)]
        for half, r in enumerate(_strassen(lambda i: wqkvt.get(7 * g + i), right)):
            qkv[par][:, _tile(half, CB)] = r

    def window(g, par):
        buf = qkv[par]
        first = lax.broadcasted_iota(jnp.int32, (DH, 128), 1) == 0
        first_row = first[0:1]

        def tile(r0, u):
            return buf[r0:r0 + DH, _tile(u)]

        for j in range(4):
            q0, k0, v0 = j * DH, 128 + j * DH, 256 + j * DH
            k = [tile(k0, t) for t in range(8)]
            v = [tile(v0, t) for t in range(8)]
            v_first = jnp.broadcast_to(buf[v0:v0 + DH, 0:1], (DH, 128))
            ks = [None] + [pltpu.roll(x, 1, 1) for x in k[1:]]
            vs = [None] + [jnp.where(first, v_first, pltpu.roll(x, 1, 1)) for x in v[1:]]
            for u in range(8):
                q = tile(q0, u) * QK_SCALE
                logits = []
                for t in range(8):
                    lg = jnp.sum(_fold8(q * (k[t] if t <= u else ks[t])), axis=0, keepdims=True)
                    if t > u:
                        lg = jnp.where(first_row, -1e9 * LOG2E, lg)
                    logits.append(lg)
                m = _tree(jnp.maximum, logits)
                p = [jnp.exp2(lg - m) for lg in logits]
                l = _tree(jnp.add, p)
                o = _tree(jnp.add, [p[t] * (v[t] if t <= u else vs[t]) for t in range(8)])
                row = pl.multiple_of(g * 128 + j * DH, DH)
                ot[2 * par + u // 4, pl.ds(row, DH), _tile(u % 4)] = (
                    o * pltpu.reciprocal(l, full_range=False))

    def layer_b(pair):
        qkv_proj(0, 0, first=True)
        window(0, 0)
        qkv_proj(0, 1, first=True)

        def b_mix(g, carry):
            window(g - 1, 1)
            qkv_proj(g, 0)
            window(g, 0)
            qkv_proj(g, 1)
            return carry
        lax.fori_loop(1, NG, b_mix, 0)
        window(NG - 1, 1)
        out_proj(wobt, 0)

        for i, form in enumerate(_right_forms(ot[2], ot[3])):
            xn.put(form, i)

        def b_out(i, carry):
            right = [xn.get(f) for f in range(7)]
            strips = [i * SPI + c for c in range(SPI)]
            for c in strips:
                rows = pl.ds(pl.multiple_of(c * 128, 128), 128)
                ys = _strassen(functools.partial(wobt.get, rows=_rows(c, 64)), right)
                for half, y in enumerate(ys):
                    b = 2 + half
                    x = xt[b, rows, :] + y
                    xt[b, rows, :] = x
                    pivot = jnp.where(c == 0, x[0:1], stats[b, 2, 0:1])
                    s1, s2 = shifted_sums(x, pivot)
                    stats[b, 0] = jnp.where(c == 0, 0.0, stats[b, 0]) + s1
                    stats[b, 1] = jnp.where(c == 0, 0.0, stats[b, 1]) + s2
                    stats[b, 2] = jnp.broadcast_to(pivot, (8, CB))
                    words = (as_bf16_bits(xt[half, rows, :]) >> 16) | as_bf16_bits(x)
                    for t in range(4):
                        xs_words[c, pl.ds(4 * half + t, 128, stride=8), :] = words[:, _tile(t)].T

            @pl.when(pair == 1)
            def _():
                for c in strips:
                    o_cp(c).start()
            return carry
        lax.fori_loop(0, 8 // SPI, b_out, 0)
        for b in (2, 3):
            put_stats(b, slice(None), stats[b, 2, 0:1], stats[b, 0], stats[b, 1])

        @pl.when(pair == 1)
        def _():
            for c in range(8):
                o_cp(c).wait()

    def as_bf16_bits(x):
        return pltpu.bitcast(x.astype(BF16).astype(F32), U32)

    def pair_body(pair, carry):
        layer_a(pair)
        layer_b(pair)
        return carry
    lax.fori_loop(0, 2, pair_body, 0)


@jax.jit
def pallas_interleave_layers__grouped_kv_mqa__sliding_local_dilated__prompt_kernel(
    A_x: jax.Array,
    A_wq: jax.Array,
    A_wk: jax.Array,
    A_wv: jax.Array,
    A_wo: jax.Array,
    B_x: jax.Array,
    B_wqkv: jax.Array,
    B_wo: jax.Array,
):
    del B_x
    hbm = pl.BlockSpec(memory_space=pl.ANY)
    vmem = pl.BlockSpec(memory_space=pltpu.VMEM)
    out = pl.pallas_call(
        _kernel,
        in_specs=[hbm, hbm, vmem, vmem, hbm, hbm, hbm],
        out_specs=hbm,
        out_shape=jax.ShapeDtypeStruct((S, D), BF16),
        scratch_shapes=[
            pltpu.VMEM((8, S, 128), BF16),
            pltpu.VMEM((D, D), BF16),
            pltpu.VMEM((D, D), BF16),
            pltpu.VMEM((D, 3 * D), BF16),
            pltpu.VMEM((D, D), BF16),
            pltpu.VMEM((DH, D), U32),
            pltpu.VMEM((7 * D // 4, D // 2), U32),
            pltpu.VMEM((7 * D // 4, D // 2), U32),
            pltpu.VMEM((NG * 7 * 96, D // 2), U32),
            pltpu.VMEM((7 * D // 4, D // 2), U32),
            pltpu.VMEM((NB, D, CB), F32),
            pltpu.VMEM((NB, 3, 8, CB), F32),
            pltpu.VMEM((2 * 7 * D // 4, CB), U32),
            pltpu.VMEM((NB * D // 2, CB), U32),
            pltpu.VMEM((NB, D, CB), F32),
            pltpu.VMEM((4 * S // 2, 128), U32),
            pltpu.VMEM((NB * DH // 2, CB), U32),
            pltpu.VMEM((S, CB), F32),
            pltpu.VMEM((384, 2 * CB), F32),
            pltpu.VMEM((384, 2 * CB), F32),
            pltpu.SemaphoreType.DMA((12,)),
        ],
        compiler_params=pltpu.CompilerParams(vmem_limit_bytes=110 * 1024 * 1024),
        name="interleave_stack",
    )(A_x.reshape(S, D), A_wq, A_wk.T, A_wv.T, A_wo, B_wqkv, B_wo)
    return out.reshape(1, S, D)
```

```python
import functools
import math

import jax
import jax.numpy as jnp
from jax import lax
import jax.experimental.pallas as pl
import jax.experimental.pallas.tpu as pltpu

S = 2048
D = 1024
DH = 32
NB = 4
CB = S // NB
NG = 8
EPS = 1e-5
LOG2E = math.log2(math.e)
QK_SCALE = DH ** -0.5 * LOG2E
KC = 256
GPI = 2
LAG = 1
MPD = 2
SPAN = 0.9
GM = 1
W0 = 1
GATE = 40
XF = 1
HOLD = 2
SPI = 2
F32 = jnp.float32
BF16 = jnp.bfloat16
U32 = jnp.uint32


def _dot(a, b):
    return jnp.dot(a, b, preferred_element_type=F32)


def _fold8(x):
    return jnp.sum(x.reshape(x.shape[0] // 8, 8, x.shape[1]), axis=0)


def _tree(op, xs):
    xs = list(xs)
    while len(xs) > 1:
        xs = [op(xs[i], xs[i + 1]) for i in range(0, len(xs), 2)]
    return xs[0]


def _tile(i, n=128):
    return slice(i * n, (i + 1) * n)


def _left_forms(a11, a12, a21, a22):
    return (a11 + a22, a21 + a22, a11, a22, a11 + a12, a21 - a11, a12 - a22)


def _right_forms(x0, x1):
    b11, b21, b12, b22 = x0[:D // 2], x0[D // 2:], x1[:D // 2], x1[D // 2:]
    forms = (b11 + b22, b11, b12 - b22, b21 - b11, b22, b11 + b12, b21 + b22)
    return [f.astype(BF16) for f in forms]


def _strassen(left, right, marks=None):
    def product(i):
        if marks is None:
            return _dot(left(i), right[i])
        a, acc = left(i), None
        for kt in range(4):
            part = _dot(a[:, _tile(kt)], right[i][_tile(kt), :])
            marks.extend(part[m:m + 8, 0:128] for m in range(0, a.shape[0], a.shape[0] // MPD))
            acc = part if acc is None else acc + part
        return acc
    m1, m2, m3, m4, m5, m6, m7 = (product(i) for i in range(7))

    def interleave(top, bottom):
        n = top.shape[0] // 16
        return jnp.concatenate(
            [top.reshape(n, 16, CB), bottom.reshape(n, 16, CB)], axis=1).reshape(32 * n, CB)
    return interleave(m1 + m4 - m5 + m7, m2 + m4), interleave(m3 + m5, m1 - m2 + m3 + m6)


class _Packed:
    def __init__(self, ref, n_rows):
        self.ref = ref
        self.n_rows = n_rows

    def _index(self, matrix, rows, cols):
        start, size = (0, self.n_rows) if rows is None else rows
        start = (matrix * self.n_rows + start) // 2
        if not isinstance(start, int):
            start = pl.multiple_of(start, 8)
        return pl.ds(start, size // 2), cols

    def get(self, matrix=0, rows=None, cols=slice(None)):
        return pltpu.bitcast(self.ref[self._index(matrix, rows, cols)], BF16)

    def put(self, value, matrix=0, rows=None, cols=slice(None)):
        self.ref[self._index(matrix, rows, cols)] = pltpu.bitcast(value.astype(BF16), U32)


def _rows(i, n=128):
    return i * n, n


def _kernel(x_hbm, wq_hbm, wkt_ref, wvt_ref, wo_hbm, wqkv_hbm, wob_hbm, out_hbm,
            xs, wq_s, wo_s, wqkv_s, wob_s, wkvt, wqt, wot, wqkvt, wobt,
            xt, stats, xn, qt, ot, kp, vt, sbuf, qkv0, qkv1, sems):
    wkvt, wqkvt, qt = _Packed(wkvt, 2 * DH), _Packed(wqkvt, 192), _Packed(qt, D)
    wqt, wot, wobt, xn, kp = (_Packed(r, CB) for r in (wqt, wot, wobt, xn, kp))
    vt = _Packed(vt, DH)
    qkv = (qkv0, qkv1)

    def x_cp(c):
        c0 = c * 128 if isinstance(c, int) else pl.multiple_of(c * 128, 128)
        return pltpu.make_async_copy(x_hbm.at[:, pl.ds(c0, 128)], xs.at[c], sems.at[c])


    def o_cp(c):
        c0 = c * 128 if isinstance(c, int) else pl.multiple_of(c * 128, 128)
        return pltpu.make_async_copy(xs.at[c], out_hbm.at[:, pl.ds(c0, 128)], sems.at[c])

    w_cp = [pltpu.make_async_copy(src, dst, sems.at[8 + i]) for i, (src, dst) in enumerate(
        [(wq_hbm, wq_s), (wo_hbm, wo_s), (wqkv_hbm, wqkv_s), (wob_hbm, wob_s)])]
    xs_words = xs.bitcast(U32)

    def shifted_sums(x, pivot):
        d = x - pivot
        return _fold8(d), _fold8(d * d)

    def put_stats(b, cols, pivot, s1, s2):
        s1 = jnp.sum(s1, axis=0, keepdims=True) * (1.0 / D)
        s2 = jnp.sum(s2, axis=0, keepdims=True) * (1.0 / D)
        rstd = lax.rsqrt(jnp.maximum(s2 - s1 * s1, 0.0) + EPS)
        stats[b, 0, :, cols] = jnp.broadcast_to(rstd, (8, rstd.shape[1]))
        stats[b, 1, :, cols] = jnp.broadcast_to((pivot + s1) * rstd, (8, rstd.shape[1]))

    def normed(b):
        return xt[b] * stats[b, 0, 0:1] - stats[b, 1, 0:1]

    def out_proj(w, par):
        ys = _strassen(w.get, _right_forms(ot[2 * par], ot[2 * par + 1]))
        for half, y in enumerate(ys):
            b = 2 * par + half
            x = xt[b] + y
            xt[b] = x
            put_stats(b, slice(None), x[0:1], *shifted_sums(x, x[0:1]))

    def prepare_weight(src, dst, base, row0, col0, kt, gate=None):
        def quarters(k0):
            t = src[pl.ds(pl.multiple_of(k0, 128), 128), pl.ds(pl.multiple_of(col0, 128), 128)]
            if gate is not None:
                w = pltpu.bitcast(t, U32).reshape(8, 8, 128) | gate
                t = pltpu.bitcast(w.reshape(64, 128), BF16)
            t = (t.astype(F32).T if XF else t.T.astype(F32)).reshape(4, 2, 16, 128)
            return t[:, 0].reshape(64, 128), t[:, 1].reshape(64, 128)
        a11, a21 = quarters(kt * 128)
        a12, a22 = quarters(kt * 128 + D // 2)
        for i, form in enumerate(_left_forms(a11, a12, a21, a22)):
            dst.put(form, base + i, rows=(row0, 64), cols=pl.ds(pl.multiple_of(kt * 128, 128), 128))

    w_cp[0].start()
    for c in range(8):
        x_cp(c).start()
    wkvt.put(wkt_ref[...], rows=_rows(0, DH))
    wkvt.put(wvt_ref[...], rows=_rows(1, DH))
    stats[...] = jnp.zeros(stats.shape, F32)

    w_cp[0].wait()

    def transpose_wq(c, carry):
        for kt in range(4):
            prepare_weight(wq_s, wqt, 0, c * 64, c * 128, kt)
        return carry
    lax.fori_loop(0, 8, transpose_wq, 0)

    def load_strip(c, carry):
        x_cp(c).wait()
        rows = pl.ds(pl.multiple_of(c * 128, 128), 128)
        for u in range(8):
            t = xs_words[c, pl.ds(u, 128, stride=8), :].T
            halves = (pltpu.bitcast(t << 16, F32), pltpu.bitcast(t & U32(0xFFFF0000), F32))
            for par, x in enumerate(halves):
                b, cols = 2 * par + u // 4, _tile(u % 4)
                xt[b, rows, cols] = x
                pivot = jnp.where(c == 0, x[0:1], stats[b, 2, :, cols])
                s1, s2 = shifted_sums(x, pivot[0:1])
                stats[b, 0, :, cols] += s1
                stats[b, 1, :, cols] += s2
                stats[b, 2, :, cols] = pivot
        return carry
    lax.fori_loop(0, 8, load_strip, 0)
    for cp in w_cp[1:]:
        cp.start()
    for b in range(NB):
        put_stats(b, slice(None), stats[b, 2], stats[b, 0], stats[b, 1])

    def other_weights(i, n):
        units = []
        for u in range(32 // n):
            c, kt = (i * (32 // n) + u) // 4, (i * (32 // n) + u) % 4
            units.append((wo_s, wot, 0, c * 64, c * 128, kt))
            units.append((wob_s, wobt, 0, c * 64, c * 128, kt))
            units += [(wqkv_s, wqkvt, 7 * c, j * 64, j * D + c * 128, kt) for j in range(3)]
        return units

    def layer_a(pair):
        lane_head = lax.broadcasted_iota(jnp.int32, (128, 128), 1) // DH

        def project(par, shift):
            xs_ = [normed(2 * par + half) for half in range(2)]
            kvs = [_dot(wkvt.get(), x.astype(BF16)) for x in xs_]
            shift = jnp.where(par == 0, jnp.mean(kvs[0][0:DH], axis=1, keepdims=True), shift)
            for half, kv in enumerate(kvs):
                b = 2 * par + half
                k = (kv[0:DH] - shift) * QK_SCALE
                vt.put(kv[DH:], b)
                for t in range(CB // 128):
                    krep = jnp.concatenate([k[:, _tile(t)]] * 4, axis=0).T
                    for j in range(4):
                        kp.put(jnp.where(lane_head == j, krep, 0.0), j * NB + b, rows=_rows(t))
            for half, q in enumerate(_strassen(wqt.get, _right_forms(*xs_))):
                qt.put(q, 2 * par + half)
            return shift
        lax.fori_loop(0, 2, project, jnp.zeros((DH, 1), F32))

        @pl.when(pair == 0)
        def _():
            for cp in w_cp[1:]:
                cp.wait()

        chunks = [(c // (CB // KC), _tile(c % (CB // KC), KC)) for c in range(S // KC)]
        n_iter = NB * NG // GPI

        def attend(i, carry):
            tot, lmin = carry
            b = i // (NG // GPI)
            g0 = (i % (NG // GPI)) * GPI
            state = {}
            units = other_weights(i, n_iter)
            zero = jnp.full((8, 128), i // 4096, jnp.int32).astype(U32)
            spots = [(u * GATE) // len(units) for u in range(len(units))]

            def pv(gi, j, c, s):
                nonlocal tot, lmin
                kb, ks = chunks[c]
                p = jnp.exp2(s)
                for unit, spot in zip(units, spots):
                    if GATE and spot == (gi * 4 + j) * len(chunks) + c:
                        prepare_weight(*unit, gate=pltpu.bitcast(p[0:8, 0:128], U32) & zero)
                acc = _dot(vt.get(kb, cols=ks), p.astype(BF16))
                l = _fold8(p)
                if c > 0:
                    acc = acc + state[gi, j][0]
                    l = l + state[gi, j][1]
                state[gi, j] = (acc, l)
                if c == len(chunks) - 1:
                    l = jnp.sum(l, axis=0, keepdims=True)
                    tot = tot + (_fold8(jnp.abs(acc)) + l)
                    lmin = jnp.minimum(lmin, l)
                    row = pl.multiple_of((g0 + gi) * 128 + j * DH, DH)
                    ot[b, pl.ds(row, DH), :] = acc * pltpu.reciprocal(l, full_range=False)

            pending = []
            for gi in range(GPI):
                q = qt.get(b, rows=((g0 + gi) * 128, 128))
                for j in range(4):
                    for c, (kb, ks) in enumerate(chunks):
                        pending.append((gi, j, c, _dot(kp.get(j * NB + kb, rows=(ks.start, KC)), q)))
                        left = 4 * GPI * len(chunks) - 1 - ((gi * 4 + j) * len(chunks) + c)
                        if len(pending) > LAG and left >= HOLD:
                            pv(*pending.pop(0))
            for item in pending:
                pv(*item)
            if not GATE:
                for unit in units:
                    prepare_weight(*unit)
            return tot, lmin

        tot, lmin = lax.fori_loop(0, n_iter, attend,
                                  (jnp.zeros((8, CB), F32), jnp.ones((1, CB), F32)))

        safe = (tot <= 2.0 ** 120) & (lmin >= 2.0 ** -30)
        n_unsafe = jnp.sum(jnp.where(safe, 0.0, 1.0))

        @pl.when(n_unsafe > 0.0)
        def _():
            def attend_true_max(i, carry):
                b = i // (4 * NG)
                h = i % (4 * NG)
                q = qt.get(b, rows=((h // 4) * 128, 128))
                for c, (kb, ks) in enumerate(chunks):
                    sbuf[_tile(c, KC), :] = _dot(kp.get(h % 4 * NB + kb, rows=(ks.start, KC)), q)
                m = jnp.max(sbuf[...], axis=0, keepdims=True)
                acc = jnp.zeros((DH, CB), F32)
                l = jnp.zeros((8, CB), F32)
                for c, (kb, ks) in enumerate(chunks):
                    p = jnp.exp2(sbuf[_tile(c, KC), :] - m)
                    acc = acc + _dot(vt.get(kb, cols=ks), p.astype(BF16))
                    l = l + _fold8(p)
                ot[b, pl.ds(pl.multiple_of(h * DH, DH), DH), :] = acc / jnp.sum(l, axis=0, keepdims=True)
                return carry
            lax.fori_loop(0, NB * 4 * NG, attend_true_max, 0)

        def a_out(par, carry):
            out_proj(wot, par)
            return carry
        lax.fori_loop(0, 2, a_out, 0)

    def qkv_proj(g, par, first=False, marks=None):
        if first:
            right = _right_forms(normed(2 * par), normed(2 * par + 1))
            for i, form in enumerate(right):
                xn.put(form, 7 * par + i)
        else:
            right = [xn.get(7 * par + i) for i in range(7)]
        for half, r in enumerate(_strassen(lambda i: wqkvt.get(7 * g + i), right, marks)):
            qkv[par][:, _tile(half, CB)] = r

    def window(g, par, marks=None):
        buf = qkv[par]
        zero = jnp.full((8, 128), g // 4096, jnp.int32).astype(U32)

        def gated(x, step):
            if marks is None:
                return x
            gate = pltpu.bitcast(marks[int(step * SPAN * len(marks) / 64)], U32) & zero
            w = pltpu.bitcast(jnp.broadcast_to(x, (max(8, x.shape[0]), 128)), U32).reshape(-1, 8, 128) | gate
            return pltpu.bitcast(w.reshape(-1, 128), F32)

        first = lax.broadcasted_iota(jnp.int32, (DH, 128), 1) == 0
        first_row = first[0:1]

        def tile(r0, u):
            return buf[r0:r0 + DH, _tile(u)]

        for j in range(4):
            q0, k0, v0 = j * DH, 128 + j * DH, 256 + j * DH
            k = [tile(k0, t) for t in range(8)]
            v = [tile(v0, t) for t in range(8)]
            v_first = jnp.broadcast_to(buf[v0:v0 + DH, 0:1], (DH, 128))
            ks = [None] + [pltpu.roll(x, 1, 1) for x in k[1:]]
            vs = [None] + [jnp.where(first, v_first, pltpu.roll(x, 1, 1)) for x in v[1:]]
            for u in range(8):
                q = tile(q0, u) * gated(jnp.full((1, 128), QK_SCALE, F32), j * 16 + 2 * u)[0:1]
                logits = []
                for t in range(8):
                    lg = jnp.sum(_fold8(q * (k[t] if t <= u else ks[t])), axis=0, keepdims=True)
                    if t > u:
                        lg = jnp.where(first_row, -1e9 * LOG2E, lg)
                    logits.append(lg)
                m = _tree(jnp.maximum, logits)
                if GM: m = gated(m, j * 16 + 2 * u + 1)[0:1]
                p = [jnp.exp2(lg - m) for lg in logits]
                l = _tree(jnp.add, p)
                o = _tree(jnp.add, [p[t] * (v[t] if t <= u else vs[t]) for t in range(8)])
                row = pl.multiple_of(g * 128 + j * DH, DH)
                ot[2 * par + u // 4, pl.ds(row, DH), _tile(u % 4)] = (
                    o * pltpu.reciprocal(l, full_range=False))

    def layer_b(pair):
        qkv_proj(0, 0, first=True)
        window(0, 0)
        qkv_proj(0, 1, first=True)

        def b_mix(g, carry):
            m0, m1 = [], []
            qkv_proj(g, 0, marks=m0 if W0 else None)
            window(g - 1, 1, m0 if W0 else None)
            qkv_proj(g, 1, marks=m1)
            window(g, 0, m1)
            return carry
        lax.fori_loop(1, NG, b_mix, 0)
        window(NG - 1, 1)
        out_proj(wobt, 0)

        for i, form in enumerate(_right_forms(ot[2], ot[3])):
            xn.put(form, i)

        def b_out(i, carry):
            right = [xn.get(f) for f in range(7)]
            strips = [i * SPI + c for c in range(SPI)]
            for c in strips:
                rows = pl.ds(pl.multiple_of(c * 128, 128), 128)
                ys = _strassen(functools.partial(wobt.get, rows=_rows(c, 64)), right)
                for half, y in enumerate(ys):
                    b = 2 + half
                    x = xt[b, rows, :] + y
                    xt[b, rows, :] = x
                    pivot = jnp.where(c == 0, x[0:1], stats[b, 2, 0:1])
                    s1, s2 = shifted_sums(x, pivot)
                    stats[b, 0] = jnp.where(c == 0, 0.0, stats[b, 0]) + s1
                    stats[b, 1] = jnp.where(c == 0, 0.0, stats[b, 1]) + s2
                    stats[b, 2] = jnp.broadcast_to(pivot, (8, CB))
                    words = (as_bf16_bits(xt[half, rows, :]) >> 16) | as_bf16_bits(x)
                    for t in range(4):
                        xs_words[c, pl.ds(4 * half + t, 128, stride=8), :] = words[:, _tile(t)].T

            @pl.when(pair == 1)
            def _():
                for c in strips:
                    o_cp(c).start()
            return carry
        lax.fori_loop(0, 8 // SPI, b_out, 0)
        for b in (2, 3):
            put_stats(b, slice(None), stats[b, 2, 0:1], stats[b, 0], stats[b, 1])

        @pl.when(pair == 1)
        def _():
            for c in range(8):
                o_cp(c).wait()

    def as_bf16_bits(x):
        return pltpu.bitcast(x.astype(BF16).astype(F32), U32)

    def pair_body(pair, carry):
        layer_a(pair)
        layer_b(pair)
        return carry
    lax.fori_loop(0, 2, pair_body, 0)


@jax.jit
def pallas_interleave_layers__grouped_kv_mqa__sliding_local_dilated__prompt_kernel(
    A_x: jax.Array,
    A_wq: jax.Array,
    A_wk: jax.Array,
    A_wv: jax.Array,
    A_wo: jax.Array,
    B_x: jax.Array,
    B_wqkv: jax.Array,
    B_wo: jax.Array,
):
    del B_x
    hbm = pl.BlockSpec(memory_space=pl.ANY)
    vmem = pl.BlockSpec(memory_space=pltpu.VMEM)
    out = pl.pallas_call(
        _kernel,
        in_specs=[hbm, hbm, vmem, vmem, hbm, hbm, hbm],
        out_specs=hbm,
        out_shape=jax.ShapeDtypeStruct((S, D), BF16),
        scratch_shapes=[
            pltpu.VMEM((8, S, 128), BF16),
            pltpu.VMEM((D, D), BF16),
            pltpu.VMEM((D, D), BF16),
            pltpu.VMEM((D, 3 * D), BF16),
            pltpu.VMEM((D, D), BF16),
            pltpu.VMEM((DH, D), U32),
            pltpu.VMEM((7 * D // 4, D // 2), U32),
            pltpu.VMEM((7 * D // 4, D // 2), U32),
            pltpu.VMEM((NG * 7 * 96, D // 2), U32),
            pltpu.VMEM((7 * D // 4, D // 2), U32),
            pltpu.VMEM((NB, D, CB), F32),
            pltpu.VMEM((NB, 3, 8, CB), F32),
            pltpu.VMEM((2 * 7 * D // 4, CB), U32),
            pltpu.VMEM((NB * D // 2, CB), U32),
            pltpu.VMEM((NB, D, CB), F32),
            pltpu.VMEM((4 * S // 2, 128), U32),
            pltpu.VMEM((NB * DH // 2, CB), U32),
            pltpu.VMEM((S, CB), F32),
            pltpu.VMEM((384, 2 * CB), F32),
            pltpu.VMEM((384, 2 * CB), F32),
            pltpu.SemaphoreType.DMA((12,)),
        ],
        compiler_params=pltpu.CompilerParams(vmem_limit_bytes=110 * 1024 * 1024),
        name="interleave_stack",
    )(A_x.reshape(S, D), A_wq, A_wk.T, A_wv.T, A_wo, B_wqkv, B_wo)
    return out.reshape(1, S, D)
```

```python
import functools
import math

import jax
import jax.numpy as jnp
from jax import lax
import jax.experimental.pallas as pl
import jax.experimental.pallas.tpu as pltpu

S = 2048
D = 1024
DH = 32
NB = 4
CB = S // NB
NG = 8
EPS = 1e-5
LOG2E = math.log2(math.e)
QK_SCALE = DH ** -0.5 * LOG2E
KC = 256
GPI = 2
LAG = 1
MPD = 4
MPO = 8
SPAN_W = 0.8
SPAN_F = 0.85
SPAN_L = 0.9
SPAN = 0.9
NQ = 4
NV = 4
GR = 0
W0 = 1
GATE = 40
DELAY = 2
XF = 1
HOLD = 2
SPI = 2
F32 = jnp.float32
BF16 = jnp.bfloat16
U32 = jnp.uint32


def _dot(a, b):
    return jnp.dot(a, b, preferred_element_type=F32)


def _fold8(x):
    return jnp.sum(x.reshape(x.shape[0] // 8, 8, x.shape[1]), axis=0)


def _tree(op, xs):
    xs = list(xs)
    while len(xs) > 1:
        xs = [op(xs[i], xs[i + 1]) for i in range(0, len(xs), 2)]
    return xs[0]


def _tile(i, n=128):
    return slice(i * n, (i + 1) * n)


def _left_forms(a11, a12, a21, a22):
    return (a11 + a22, a21 + a22, a11, a22, a11 + a12, a21 - a11, a12 - a22)


def _heads_on_sublanes(x):
    x = x.reshape(8, 2, 8, x.shape[1])
    return [x[:, j].swapaxes(0, 1).reshape(64, x.shape[-1]) for j in range(2)]


def _right_forms(x0, x1):
    n = x0.shape[0] // 2
    b11, b21, b12, b22 = x0[:n], x0[n:], x1[:n], x1[n:]
    forms = (b11 + b22, b11, b12 - b22, b21 - b11, b22, b11 + b12, b21 + b22)
    return [f.astype(BF16) for f in forms]


def _strassen(left, right, marks=None, per_dot=2, interleaved=True):
    def product(i):
        if marks is None:
            return _dot(left(i), right[i])
        a, acc = left(i), None
        for kt in range(4):
            part = _dot(a[:, _tile(kt)], right[i][_tile(kt), :])
            marks.extend(part[m:m + 8, 0:128] for m in range(0, a.shape[0], a.shape[0] // per_dot))
            acc = part if acc is None else acc + part
        return acc
    m1, m2, m3, m4, m5, m6, m7 = (product(i) for i in range(7))

    def interleave(top, bottom):
        if not interleaved:
            return jnp.concatenate([top, bottom], axis=0)
        n = top.shape[0] // 16
        return jnp.concatenate(
            [top.reshape(n, 16, CB), bottom.reshape(n, 16, CB)], axis=1).reshape(32 * n, CB)
    return interleave(m1 + m4 - m5 + m7, m2 + m4), interleave(m3 + m5, m1 - m2 + m3 + m6)


class _Packed:
    def __init__(self, ref, n_rows):
        self.ref = ref
        self.n_rows = n_rows

    def _index(self, matrix, rows, cols):
        start, size = (0, self.n_rows) if rows is None else rows
        start = (matrix * self.n_rows + start) // 2
        if not isinstance(start, int):
            start = pl.multiple_of(start, 8)
        return pl.ds(start, size // 2), cols

    def get(self, matrix=0, rows=None, cols=slice(None)):
        return pltpu.bitcast(self.ref[self._index(matrix, rows, cols)], BF16)

    def put(self, value, matrix=0, rows=None, cols=slice(None)):
        self.ref[self._index(matrix, rows, cols)] = pltpu.bitcast(value.astype(BF16), U32)


def _rows(i, n=128):
    return i * n, n


def _kernel(x_hbm, wq_hbm, wkt_ref, wvt_ref, wo_hbm, wqkv_hbm, wob_hbm, out_hbm,
            xs, wq_s, wo_s, wqkv_s, wob_s, wkvt, wqt, wot, wqkvt, wobt,
            xt, stats, xn, qt, ot, kp, vt, sbuf, qkv0, qkv1, sems):
    wkvt, wqkvt, qt = _Packed(wkvt, 2 * DH), _Packed(wqkvt, 192), _Packed(qt, D)
    wqt, wot, wobt, xn, kp = (_Packed(r, CB) for r in (wqt, wot, wobt, xn, kp))
    vt = _Packed(vt, DH)
    qkv = (qkv0, qkv1)

    def x_cp(c):
        c0 = c * 128 if isinstance(c, int) else pl.multiple_of(c * 128, 128)
        return pltpu.make_async_copy(x_hbm.at[:, pl.ds(c0, 128)], xs.at[c], sems.at[c])


    def o_cp(c):
        c0 = c * 128 if isinstance(c, int) else pl.multiple_of(c * 128, 128)
        return pltpu.make_async_copy(xs.at[c], out_hbm.at[:, pl.ds(c0, 128)], sems.at[c])

    w_cp = [pltpu.make_async_copy(src, dst, sems.at[8 + i]) for i, (src, dst) in enumerate(
        [(wq_hbm, wq_s), (wo_hbm, wo_s), (wqkv_hbm, wqkv_s), (wob_hbm, wob_s)])]
    xs_words = xs.bitcast(U32)

    def shifted_sums(x, pivot):
        d = x - pivot
        return _fold8(d), _fold8(d * d)

    def put_stats(b, cols, pivot, s1, s2):
        s1 = jnp.sum(s1, axis=0, keepdims=True) * (1.0 / D)
        s2 = jnp.sum(s2, axis=0, keepdims=True) * (1.0 / D)
        rstd = lax.rsqrt(jnp.maximum(s2 - s1 * s1, 0.0) + EPS)
        stats[b, 0, :, cols] = jnp.broadcast_to(rstd, (8, rstd.shape[1]))
        stats[b, 1, :, cols] = jnp.broadcast_to((pivot + s1) * rstd, (8, rstd.shape[1]))

    def normed(b):
        return xt[b] * stats[b, 0, 0:1] - stats[b, 1, 0:1]

    def gated(x, marks, frac, zero):
        if marks is None:
            return x
        gate = pltpu.bitcast(marks[int(frac * len(marks))], U32) & zero
        x = jnp.broadcast_to(x, (max(8, x.shape[0]), 128))
        return pltpu.bitcast((pltpu.bitcast(x, U32).reshape(-1, 8, 128) | gate).reshape(-1, 128), F32)

    def out_proj(w, par, marks=None):
        ys = _strassen(w.get, _right_forms(ot[2 * par], ot[2 * par + 1]), marks, MPO if marks is not None else 0)
        for half, y in enumerate(ys):
            b = 2 * par + half
            x = xt[b] + y
            xt[b] = x
            put_stats(b, slice(None), x[0:1], *shifted_sums(x, x[0:1]))

    def prepare_steps(src, dst, base, row0, col0, kt):
        st = {}

        def load(half, gate=None):
            k0 = pl.multiple_of(kt * 128 + half * (D // 2), 128)
            t = src[pl.ds(k0, 128), pl.ds(pl.multiple_of(col0, 128), 128)]
            if gate is not None:
                w = pltpu.bitcast(t, U32).reshape(8, 8, 128) | gate
                t = pltpu.bitcast(w.reshape(64, 128), BF16)
            if src is wob_s:
                t = jnp.concatenate(_heads_on_sublanes(t.astype(F32)), axis=0).T
            else:
                t = t.T.astype(F32)
            st[half] = t

        def split(half, gate=None):
            t = st[half]
            if gate is not None and src is wqkv_s:
                w = pltpu.bitcast(t, U32).reshape(16, 8, 128) | gate
                t = pltpu.bitcast(w.reshape(128, 128), F32)
            if src is wqkv_s:
                st[half] = _heads_on_sublanes(t)
            else:
                t = t.reshape(4, 2, 16, 128)
                st[half] = (t[:, 0].reshape(64, 128), t[:, 1].reshape(64, 128))

        def store(gate=None):
            (a11, a21), (a12, a22) = st[0], st[1]
            for i, form in enumerate(_left_forms(a11, a12, a21, a22)):
                dst.put(form, base + i, rows=(row0, 64), cols=pl.ds(pl.multiple_of(kt * 128, 128), 128))

        P = functools.partial
        return [(0, P(load, 0)), (1, P(split, 0)), (1, P(load, 1)), (2, P(split, 1)), (2, store)]

    w_cp[0].start()
    for c in range(8):
        x_cp(c).start()
    wkvt.put(wkt_ref[...], rows=_rows(0, DH))
    wkvt.put(wvt_ref[...], rows=_rows(1, DH))
    stats[...] = jnp.zeros(stats.shape, F32)

    w_cp[0].wait()

    def transpose_wq(c, carry):
        for kt in range(4):
            for _, step in prepare_steps(wq_s, wqt, 0, c * 64, c * 128, kt):
                step()
        return carry
    lax.fori_loop(0, 8, transpose_wq, 0)

    def load_strip(c, carry):
        x_cp(c).wait()
        rows = pl.ds(pl.multiple_of(c * 128, 128), 128)
        for u in range(8):
            t = xs_words[c, pl.ds(u, 128, stride=8), :].T
            halves = (pltpu.bitcast(t << 16, F32), pltpu.bitcast(t & U32(0xFFFF0000), F32))
            for par, x in enumerate(halves):
                b, cols = 2 * par + u // 4, _tile(u % 4)
                xt[b, rows, cols] = x
                pivot = jnp.where(c == 0, x[0:1], stats[b, 2, :, cols])
                s1, s2 = shifted_sums(x, pivot[0:1])
                stats[b, 0, :, cols] += s1
                stats[b, 1, :, cols] += s2
                stats[b, 2, :, cols] = pivot
        return carry
    lax.fori_loop(0, 8, load_strip, 0)
    for cp in w_cp[1:]:
        cp.start()
    for b in range(NB):
        put_stats(b, slice(None), stats[b, 2], stats[b, 0], stats[b, 1])

    def other_weights(i, n):
        units = []
        for u in range(32 // n):
            c, kt = (i * (32 // n) + u) // 4, (i * (32 // n) + u) % 4
            units.append((wo_s, wot, 0, c * 64, c * 128, kt))
            units.append((wob_s, wobt, 0, c * 64, c * 128, kt))
            units += [(wqkv_s, wqkvt, 7 * c, j * 64, j * D + c * 128, kt) for j in range(3)]
        return units

    def layer_a(pair):
        lane_head = lax.broadcasted_iota(jnp.int32, (128, 128), 1) // DH

        def project(par, shift):
            xs_ = [normed(2 * par + half) for half in range(2)]
            kvs = [_dot(wkvt.get(), x.astype(BF16)) for x in xs_]
            shift = jnp.where(par == 0, jnp.mean(kvs[0][0:DH], axis=1, keepdims=True), shift)
            for half, kv in enumerate(kvs):
                b = 2 * par + half
                k = (kv[0:DH] - shift) * QK_SCALE
                vt.put(kv[DH:], b)
                for t in range(CB // 128):
                    krep = jnp.concatenate([k[:, _tile(t)]] * 4, axis=0).T
                    for j in range(4):
                        kp.put(jnp.where(lane_head == j, krep, 0.0), j * NB + b, rows=_rows(t))
            for half, q in enumerate(_strassen(wqt.get, _right_forms(*xs_))):
                qt.put(q, 2 * par + half)
            return shift
        lax.fori_loop(0, 2, project, jnp.zeros((DH, 1), F32))

        @pl.when(pair == 0)
        def _():
            for cp in w_cp[1:]:
                cp.wait()

        chunks = [(c // (CB // KC), _tile(c % (CB // KC), KC)) for c in range(S // KC)]
        n_iter = NB * NG // GPI

        def attend(i, carry):
            tot, lmin = carry
            b = i // (NG // GPI)
            g0 = (i % (NG // GPI)) * GPI
            state = {}
            units = other_weights(i, n_iter)
            zero = jnp.full((8, 128), i // 4096, jnp.int32).astype(U32)
            steps = [((u * GATE) // len(units) + d * DELAY, step)
                     for u, unit in enumerate(units) for d, step in prepare_steps(*unit)]

            def pv(gi, j, c, s):
                nonlocal tot, lmin
                kb, ks = chunks[c]
                p = jnp.exp2(s)
                for spot, step in steps:
                    if spot == (gi * 4 + j) * len(chunks) + c:
                        step(pltpu.bitcast(p[0:8, 0:128], U32) & zero)
                acc = _dot(vt.get(kb, cols=ks), p.astype(BF16))
                l = _fold8(p)
                if c > 0:
                    acc = acc + state[gi, j][0]
                    l = l + state[gi, j][1]
                state[gi, j] = (acc, l)
                if c == len(chunks) - 1:
                    l = jnp.sum(l, axis=0, keepdims=True)
                    tot = tot + (_fold8(jnp.abs(acc)) + l)
                    lmin = jnp.minimum(lmin, l)
                    row = pl.multiple_of((g0 + gi) * 128 + j * DH, DH)
                    ot[b, pl.ds(row, DH), :] = acc * pltpu.reciprocal(l, full_range=False)

            pending = []
            for gi in range(GPI):
                q = qt.get(b, rows=((g0 + gi) * 128, 128))
                for j in range(4):
                    for c, (kb, ks) in enumerate(chunks):
                        pending.append((gi, j, c, _dot(kp.get(j * NB + kb, rows=(ks.start, KC)), q)))
                        left = 4 * GPI * len(chunks) - 1 - ((gi * 4 + j) * len(chunks) + c)
                        if len(pending) > LAG and left >= HOLD:
                            pv(*pending.pop(0))
            for item in pending:
                pv(*item)
            return tot, lmin

        tot, lmin = lax.fori_loop(0, n_iter, attend,
                                  (jnp.zeros((8, CB), F32), jnp.ones((1, CB), F32)))

        safe = (tot <= 2.0 ** 120) & (lmin >= 2.0 ** -30)
        n_unsafe = jnp.sum(jnp.where(safe, 0.0, 1.0))

        @pl.when(n_unsafe > 0.0)
        def _():
            def attend_true_max(i, carry):
                b = i // (4 * NG)
                h = i % (4 * NG)
                q = qt.get(b, rows=((h // 4) * 128, 128))
                for c, (kb, ks) in enumerate(chunks):
                    sbuf[_tile(c, KC), :] = _dot(kp.get(h % 4 * NB + kb, rows=(ks.start, KC)), q)
                m = jnp.max(sbuf[...], axis=0, keepdims=True)
                acc = jnp.zeros((DH, CB), F32)
                l = jnp.zeros((8, CB), F32)
                for c, (kb, ks) in enumerate(chunks):
                    p = jnp.exp2(sbuf[_tile(c, KC), :] - m)
                    acc = acc + _dot(vt.get(kb, cols=ks), p.astype(BF16))
                    l = l + _fold8(p)
                ot[b, pl.ds(pl.multiple_of(h * DH, DH), DH), :] = acc / jnp.sum(l, axis=0, keepdims=True)
                return carry
            lax.fori_loop(0, NB * 4 * NG, attend_true_max, 0)

        def a_out(par, carry):
            out_proj(wot, par)
            return carry
        lax.fori_loop(0, 2, a_out, 0)

    def qkv_proj(g, par, first=False, marks=None):
        if first:
            right = _right_forms(normed(2 * par), normed(2 * par + 1))
            for i, form in enumerate(right):
                xn.put(form, 7 * par + i)
        else:
            right = [xn.get(7 * par + i) for i in range(7)]
        for half, r in enumerate(_strassen(lambda i: wqkvt.get(7 * g + i), right, marks, MPD, False)):
            qkv[par][:, _tile(half, CB)] = r

    def window(pair, g, par, marks=None, span=SPAN):
        buf = qkv[par]
        zero = jnp.full((8, 128), pair // 4096, jnp.int32).astype(U32)
        first = lax.broadcasted_iota(jnp.int32, (128, 128), 1) == 0
        even = lax.broadcasted_iota(jnp.int32, (8, 128), 0) % 2 == 0

        def paced(x, step):
            return gated(x, marks, span * step, zero)

        def tile(kind, u):
            return jnp.concatenate([buf[r:r + 64, _tile(u)] for r in (kind * 64, 192 + kind * 64)])

        k = [tile(1, t) for t in range(8)]
        v = [tile(2, t) for t in range(8)]
        v_first = jnp.broadcast_to(v[0][:, 0:1], (128, 128))
        ks = [None] + [pltpu.roll(x, 1, 1) for x in k[1:]]
        vs = [None] + [jnp.where(first, v_first, pltpu.roll(x, 1, 1)) for x in v[1:]]
        if GR:
            ks = [None] + [pltpu.roll(paced(x, (t - 1) / 8), 1, 1) for t, x in enumerate(k) if t]
        for u in range(8):
            q = tile(0, u).reshape(16, 8, 128)
            logits = []
            for t in range(8):
                if t % (8 // NQ) == 0:
                    scale = paced(jnp.full((8, 128), QK_SCALE, F32), (u + 0.5 * t / 8) / 8)
                    qs = q * scale
                lg = jnp.sum(qs * (k[t] if t <= u else ks[t]).reshape(16, 8, 128), axis=0)
                lg = lg + jnp.where(even, pltpu.roll(lg, 7, 0), pltpu.roll(lg, 1, 0))
                if t > u:
                    lg = jnp.where(first[0:8], -1e9 * LOG2E, lg)
                logits.append(lg)
            m = _tree(jnp.maximum, logits)
            p = [jnp.exp2(lg - m) for lg in logits]
            inv = pltpu.reciprocal(_tree(jnp.add, p), full_range=False)
            n = 16 // NV
            for part in range(NV):
                r = paced(inv, (u + 0.5 + 0.5 * part / NV) / 8)
                o = None
                for t in range(8):
                    x = (v[t] if t <= u else vs[t]).reshape(16, 8, 128)[part * n:(part + 1) * n]
                    pv = (p[t] * r) * x
                    o = pv if o is None else o + pv
                rows = pl.ds(pl.multiple_of(g * 128 + part * n * 8, n * 8), n * 8)
                ot[2 * par + u // 4, rows, _tile(u % 4)] = o.reshape(n * 8, 128)

    def layer_b(pair):
        qkv_proj(0, 0, first=True)
        marks = []
        qkv_proj(0, 1, first=True, marks=marks)
        window(pair, 0, 0, marks)

        def b_mix(g, carry):
            m0, m1 = [], []
            qkv_proj(g, 0, marks=m0)
            window(pair, g - 1, 1, m0)
            qkv_proj(g, 1, marks=m1)
            window(pair, g, 0, m1)
            return carry
        lax.fori_loop(1, NG, b_mix, 0)
        marks = []
        out_proj(wobt, 0, marks)
        window(pair, NG - 1, 1, marks, SPAN_W)

        zero = jnp.full((8, 128), pair // 4096, jnp.int32).astype(U32)
        for n, (kt, t) in enumerate((kt, t) for kt in range(4) for t in range(4)):
            frac = SPAN_F * n / 12 if kt < 3 else SPAN_L
            xs_ = [jnp.concatenate([gated(ot[b, _tile(k), _tile(t)], marks, frac, zero)
                                    for k in (kt, kt + 4)]) for b in (2, 3)]
            for i, form in enumerate(_right_forms(*xs_)):
                xn.put(form, i, rows=_rows(kt), cols=_tile(t))

        def b_out(i, carry):
            right = [xn.get(f) for f in range(7)]
            strips = [i * SPI + c for c in range(SPI)]
            for c in strips:
                rows = pl.ds(pl.multiple_of(c * 128, 128), 128)
                ys = _strassen(functools.partial(wobt.get, rows=_rows(c, 64)), right)
                for half, y in enumerate(ys):
                    b = 2 + half
                    x = xt[b, rows, :] + y
                    xt[b, rows, :] = x
                    pivot = jnp.where(c == 0, x[0:1], stats[b, 2, 0:1])
                    s1, s2 = shifted_sums(x, pivot)
                    stats[b, 0] = jnp.where(c == 0, 0.0, stats[b, 0]) + s1
                    stats[b, 1] = jnp.where(c == 0, 0.0, stats[b, 1]) + s2
                    stats[b, 2] = jnp.broadcast_to(pivot, (8, CB))
                    words = (as_bf16_bits(xt[half, rows, :]) >> 16) | as_bf16_bits(x)
                    for t in range(4):
                        xs_words[c, pl.ds(4 * half + t, 128, stride=8), :] = words[:, _tile(t)].T

            @pl.when(pair == 1)
            def _():
                for c in strips:
                    o_cp(c).start()
            return carry
        lax.fori_loop(0, 8 // SPI, b_out, 0)
        for b in (2, 3):
            put_stats(b, slice(None), stats[b, 2, 0:1], stats[b, 0], stats[b, 1])

        @pl.when(pair == 1)
        def _():
            for c in range(8):
                o_cp(c).wait()

    def as_bf16_bits(x):
        return pltpu.bitcast(x.astype(BF16).astype(F32), U32)

    def pair_body(pair, carry):
        layer_a(pair)
        layer_b(pair)
        return carry
    lax.fori_loop(0, 2, pair_body, 0)


@jax.jit
def pallas_interleave_layers__grouped_kv_mqa__sliding_local_dilated__prompt_kernel(
    A_x: jax.Array,
    A_wq: jax.Array,
    A_wk: jax.Array,
    A_wv: jax.Array,
    A_wo: jax.Array,
    B_x: jax.Array,
    B_wqkv: jax.Array,
    B_wo: jax.Array,
):
    del B_x
    hbm = pl.BlockSpec(memory_space=pl.ANY)
    vmem = pl.BlockSpec(memory_space=pltpu.VMEM)
    out = pl.pallas_call(
        _kernel,
        in_specs=[hbm, hbm, vmem, vmem, hbm, hbm, hbm],
        out_specs=hbm,
        out_shape=jax.ShapeDtypeStruct((S, D), BF16),
        scratch_shapes=[
            pltpu.VMEM((8, S, 128), BF16),
            pltpu.VMEM((D, D), BF16),
            pltpu.VMEM((D, D), BF16),
            pltpu.VMEM((D, 3 * D), BF16),
            pltpu.VMEM((D, D), BF16),
            pltpu.VMEM((DH, D), U32),
            pltpu.VMEM((7 * D // 4, D // 2), U32),
            pltpu.VMEM((7 * D // 4, D // 2), U32),
            pltpu.VMEM((NG * 7 * 96, D // 2), U32),
            pltpu.VMEM((7 * D // 4, D // 2), U32),
            pltpu.VMEM((NB, D, CB), F32),
            pltpu.VMEM((NB, 3, 8, CB), F32),
            pltpu.VMEM((2 * 7 * D // 4, CB), U32),
            pltpu.VMEM((NB * D // 2, CB), U32),
            pltpu.VMEM((NB, D, CB), F32),
            pltpu.VMEM((4 * S // 2, 128), U32),
            pltpu.VMEM((NB * DH // 2, CB), U32),
            pltpu.VMEM((S, CB), F32),
            pltpu.VMEM((384, 2 * CB), F32),
            pltpu.VMEM((384, 2 * CB), F32),
            pltpu.SemaphoreType.DMA((12,)),
        ],
        compiler_params=pltpu.CompilerParams(vmem_limit_bytes=110 * 1024 * 1024),
        name="interleave_stack",
    )(A_x.reshape(S, D), A_wq, A_wk.T, A_wv.T, A_wo, B_wqkv, B_wo)
    return out.reshape(1, S, D)
```

```python
import functools
import math

import jax
import jax.numpy as jnp
from jax import lax
import jax.experimental.pallas as pl
import jax.experimental.pallas.tpu as pltpu

S = 2048
D = 1024
DH = 32
NB = 4
CB = S // NB
NG = 8
EPS = 1e-5
LOG2E = math.log2(math.e)
QK_SCALE = DH ** -0.5 * LOG2E
KC = 256
GPI = 2
LAG = 1
MPD = 4
NSP = 4
NV_KEYS = 64
VG = 1
VSPLIT = 4
VGATE = 1
DL = 0.05
LW = 4
PSPLIT = 0
MPO = 8
SPAN_W = 0.75
SPAN_F = 0.85
SPAN_L = 0.8
SPAN = 0.9
NQ = 4
NV = 4
GR = 0
W0 = 1
GATE = 40
DELAY = 2
XF = 1
HOLD = 2
SPI = 2
F32 = jnp.float32
BF16 = jnp.bfloat16
U32 = jnp.uint32


def _dot(a, b):
    return jnp.dot(a, b, preferred_element_type=F32)


def _fold8(x):
    return jnp.sum(x.reshape(x.shape[0] // 8, 8, x.shape[1]), axis=0)


def _tree(op, xs):
    xs = list(xs)
    while len(xs) > 1:
        xs = [op(xs[i], xs[i + 1]) for i in range(0, len(xs), 2)]
    return xs[0]


def _tile(i, n=128):
    return slice(i * n, (i + 1) * n)


def _left_forms(a11, a12, a21, a22):
    return (a11 + a22, a21 + a22, a11, a22, a11 + a12, a21 - a11, a12 - a22)


def _heads_on_sublanes(x):
    x = x.reshape(8, 2, 8, x.shape[1])
    return [x[:, j].swapaxes(0, 1).reshape(64, x.shape[-1]) for j in range(2)]


def _right_forms(x0, x1):
    n = x0.shape[0] // 2
    b11, b21, b12, b22 = x0[:n], x0[n:], x1[:n], x1[n:]
    forms = (b11 + b22, b11, b12 - b22, b21 - b11, b22, b11 + b12, b21 + b22)
    return [f.astype(BF16) for f in forms]


def _strassen(left, right, marks=None, per_dot=2, interleaved=True, n_split=7):
    def product(i):
        if marks is None or i >= n_split:
            return _dot(left(i), right[i])
        a, acc = left(i), None
        for kt in range(4):
            part = _dot(a[:, _tile(kt)], right[i][_tile(kt), :])
            marks.extend(part[m:m + 8, 0:128] for m in range(0, a.shape[0], a.shape[0] // per_dot))
            acc = part if acc is None else acc + part
        return acc
    m1, m2, m3, m4, m5, m6, m7 = (product(i) for i in range(7))

    def interleave(top, bottom):
        if not interleaved:
            return jnp.concatenate([top, bottom], axis=0)
        n = top.shape[0] // 16
        return jnp.concatenate(
            [top.reshape(n, 16, CB), bottom.reshape(n, 16, CB)], axis=1).reshape(32 * n, CB)
    return interleave(m1 + m4 - m5 + m7, m2 + m4), interleave(m3 + m5, m1 - m2 + m3 + m6)


class _Packed:
    def __init__(self, ref, n_rows):
        self.ref = ref
        self.n_rows = n_rows

    def _index(self, matrix, rows, cols):
        start, size = (0, self.n_rows) if rows is None else rows
        start = (matrix * self.n_rows + start) // 2
        if not isinstance(start, int):
            start = pl.multiple_of(start, 8)
        return pl.ds(start, size // 2), cols

    def get(self, matrix=0, rows=None, cols=slice(None)):
        return pltpu.bitcast(self.ref[self._index(matrix, rows, cols)], BF16)

    def put(self, value, matrix=0, rows=None, cols=slice(None)):
        self.ref[self._index(matrix, rows, cols)] = pltpu.bitcast(value.astype(BF16), U32)


def _rows(i, n=128):
    return i * n, n


def _kernel(x_hbm, wq_hbm, wkt_ref, wvt_ref, wo_hbm, wqkv_hbm, wob_hbm, out_hbm,
            xs, wq_s, wo_s, wqkv_s, wob_s, wkvt, wqt, wot, wqkvt, wobt,
            xt, stats, xn, qt, qf, kb_ref, ot, kp, vt, sbuf, qkv0, qkv1, sems):
    wkvt, wqkvt, qt = _Packed(wkvt, 2 * DH), _Packed(wqkvt, 192), _Packed(qt, D)
    wqt, wot, wobt, xn, kp = (_Packed(r, CB) for r in (wqt, wot, wobt, xn, kp))
    vt = _Packed(vt, DH)
    qkv = (qkv0, qkv1)

    def x_cp(c):
        c0 = c * 128 if isinstance(c, int) else pl.multiple_of(c * 128, 128)
        return pltpu.make_async_copy(x_hbm.at[:, pl.ds(c0, 128)], xs.at[c], sems.at[c])


    def o_cp(c):
        c0 = c * 128 if isinstance(c, int) else pl.multiple_of(c * 128, 128)
        return pltpu.make_async_copy(xs.at[c], out_hbm.at[:, pl.ds(c0, 128)], sems.at[c])

    w_cp = [pltpu.make_async_copy(src, dst, sems.at[8 + i]) for i, (src, dst) in enumerate(
        [(wq_hbm, wq_s), (wo_hbm, wo_s), (wqkv_hbm, wqkv_s), (wob_hbm, wob_s)])]
    xs_words = xs.bitcast(U32)

    def shifted_sums(x, pivot):
        d = x - pivot
        n = d.shape[0] // LW
        parts = [d[i * n:(i + 1) * n] for i in range(LW)]
        return _tree(jnp.add, map(_fold8, parts)), _tree(jnp.add, [_fold8(y * y) for y in parts])

    def put_stats(b, cols, pivot, s1, s2):
        s1 = jnp.sum(s1, axis=0, keepdims=True) * (1.0 / D)
        s2 = jnp.sum(s2, axis=0, keepdims=True) * (1.0 / D)
        rstd = lax.rsqrt(jnp.maximum(s2 - s1 * s1, 0.0) + EPS)
        stats[b, 0, :, cols] = jnp.broadcast_to(rstd, (8, rstd.shape[1]))
        stats[b, 1, :, cols] = jnp.broadcast_to((pivot + s1) * rstd, (8, rstd.shape[1]))

    def normed(b):
        return xt[b] * stats[b, 0, 0:1] - stats[b, 1, 0:1]

    def gated(x, marks, frac, zero):
        if marks is None:
            return x
        gate = pltpu.bitcast(marks[int(frac * len(marks))], U32) & zero
        x = jnp.broadcast_to(x, (max(8, x.shape[0]), 128))
        return pltpu.bitcast((pltpu.bitcast(x, U32).reshape(-1, 8, 128) | gate).reshape(-1, 128), F32)

    def out_proj(w, par, marks=None):
        ys = _strassen(w.get, _right_forms(ot[2 * par], ot[2 * par + 1]), marks, MPO, True, NSP)
        for half, y in enumerate(ys):
            b = 2 * par + half
            x = xt[b] + y
            xt[b] = x
            put_stats(b, slice(None), x[0:1], *shifted_sums(x, x[0:1]))

    def prepare_steps(src, dst, base, row0, col0, kt):
        st = {}

        def load(half, gate=None):
            k0 = pl.multiple_of(kt * 128 + half * (D // 2), 128)
            t = src[pl.ds(k0, 128), pl.ds(pl.multiple_of(col0, 128), 128)]
            if gate is not None:
                w = pltpu.bitcast(t, U32).reshape(8, 8, 128) | gate
                t = pltpu.bitcast(w.reshape(64, 128), BF16)
            if src is wob_s:
                t = jnp.concatenate(_heads_on_sublanes(t.astype(F32)), axis=0).T
            else:
                t = t.T.astype(F32)
            st[half] = t

        def split(half, gate=None):
            t = st[half]
            if gate is not None and src is wqkv_s:
                w = pltpu.bitcast(t, U32).reshape(16, 8, 128) | gate
                t = pltpu.bitcast(w.reshape(128, 128), F32)
            if src is wqkv_s:
                st[half] = _heads_on_sublanes(t)
            else:
                t = t.reshape(4, 2, 16, 128)
                st[half] = (t[:, 0].reshape(64, 128), t[:, 1].reshape(64, 128))

        def store(gate=None):
            (a11, a21), (a12, a22) = st[0], st[1]
            for i, form in enumerate(_left_forms(a11, a12, a21, a22)):
                dst.put(form, base + i, rows=(row0, 64), cols=pl.ds(pl.multiple_of(kt * 128, 128), 128))

        P = functools.partial
        return [(0, P(load, 0)), (1, P(split, 0)), (1, P(load, 1)), (2, P(split, 1)), (2, store)]

    w_cp[0].start()
    for c in range(8):
        x_cp(c).start()
    wkvt.put(wkt_ref[...], rows=_rows(0, DH))
    wkvt.put(wvt_ref[...], rows=_rows(1, DH))
    stats[...] = jnp.zeros(stats.shape, F32)

    w_cp[0].wait()

    def transpose_wq(c, carry):
        for kt in range(4):
            for _, step in prepare_steps(wq_s, wqt, 0, c * 64, c * 128, kt):
                step()
        return carry
    lax.fori_loop(0, 8, transpose_wq, 0)

    def load_strip(c, carry):
        x_cp(c).wait()
        rows = pl.ds(pl.multiple_of(c * 128, 128), 128)
        for u in range(8):
            t = xs_words[c, pl.ds(u, 128, stride=8), :].T
            halves = (pltpu.bitcast(t << 16, F32), pltpu.bitcast(t & U32(0xFFFF0000), F32))
            for par, x in enumerate(halves):
                b, cols = 2 * par + u // 4, _tile(u % 4)
                xt[b, rows, cols] = x
                pivot = jnp.where(c == 0, x[0:1], stats[b, 2, :, cols])
                s1, s2 = shifted_sums(x, pivot[0:1])
                stats[b, 0, :, cols] += s1
                stats[b, 1, :, cols] += s2
                stats[b, 2, :, cols] = pivot
        return carry
    lax.fori_loop(0, 8, load_strip, 0)
    for cp in w_cp[1:]:
        cp.start()
    for b in range(NB):
        put_stats(b, slice(None), stats[b, 2], stats[b, 0], stats[b, 1])

    def other_weights(i, n):
        units = []
        for u in range(32 // n):
            c, kt = (i * (32 // n) + u) // 4, (i * (32 // n) + u) % 4
            units.append((wo_s, wot, 0, c * 64, c * 128, kt))
            units.append((wob_s, wobt, 0, c * 64, c * 128, kt))
            units += [(wqkv_s, wqkvt, 7 * c, j * 64, j * D + c * 128, kt) for j in range(3)]
        return units

    def layer_a(pair):
        lane_head = lax.broadcasted_iota(jnp.int32, (64, 128), 1) // DH

        def project(par, shift):
            xs_ = [normed(2 * par + half) for half in range(2)]
            kvs = [_dot(wkvt.get(), x.astype(BF16)) for x in xs_]
            shift = jnp.where(par == 0, jnp.mean(kvs[0][0:DH], axis=1, keepdims=True), shift)
            for half, kv in enumerate(kvs):
                b = 2 * par + half
                k = (kv[0:DH] - shift) * QK_SCALE
                vt.put(kv[DH:], b)
                for t in range(CB // 128):
                    krep = jnp.concatenate([k[:, _tile(t)]] * 4, axis=0).T
                    words = pltpu.bitcast(krep.astype(BF16), U32)
                    if half == 1 and t == CB // 128 - 1:
                        for d in range(DH):
                            kb_ref[d] = jnp.broadcast_to(krep[128 - NV_KEYS:, d:d + 1], (NV_KEYS, 128))
                    for j in range(4):
                        kp.ref[pl.ds(pl.multiple_of((j * NB + b) * (CB // 2) + t * 64, 64), 64), :] = (
                            jnp.where(lane_head == j, words, U32(0)))
            for half, q in enumerate(_strassen(wqt.get, _right_forms(*xs_), [] if PSPLIT else None)):
                qt.put(q, 2 * par + half)
                qf[pl.ds(pl.multiple_of((2 * par + half) * D, D), D), :] = q
            return shift
        lax.fori_loop(0, 2, project, jnp.zeros((DH, 1), F32))

        @pl.when(pair == 0)
        def _():
            for cp in w_cp[1:]:
                cp.wait()

        chunks = [(c // (CB // KC), _tile(c % (CB // KC), KC)) for c in range(S // KC)]
        n_iter = NB * NG // GPI

        def attend(i, carry):
            tot, lmin = carry
            b = i // (NG // GPI)
            g0 = (i % (NG // GPI)) * GPI
            state = {}
            units = other_weights(i, n_iter)
            zero = jnp.full((8, 128), i // 4096, jnp.int32).astype(U32)
            steps = [((u * GATE) // len(units) + d * DELAY, step)
                     for u, unit in enumerate(units) for d, step in prepare_steps(*unit)]

            def pv(gi, j, c, s):
                nonlocal tot, lmin
                kb, ks = chunks[c]
                p = jnp.exp2(s)
                for spot, step in steps:
                    if spot == (gi * 4 + j) * len(chunks) + c:
                        step(pltpu.bitcast(p[0:8, 0:128], U32) & zero)
                acc = _dot(vt.get(kb, cols=ks), p.astype(BF16))
                l = _fold8(p)
                if c > 0:
                    acc = acc + state[gi, j][0]
                    l = l + state[gi, j][1]
                state[gi, j] = (acc, l)
                if c == len(chunks) - 1:
                    l = jnp.sum(l, axis=0, keepdims=True)
                    tot = tot + (_fold8(jnp.abs(acc)) + l)
                    lmin = jnp.minimum(lmin, l)
                    row = pl.multiple_of((g0 + gi) * 128 + j * DH, DH)
                    ot[b, pl.ds(row, DH), :] = acc * pltpu.reciprocal(l, full_range=False)

            pending = []
            n_pieces = NV_KEYS // (8 * VG) * VSPLIT
            for gi in range(GPI):
                q = qt.get(b, rows=((g0 + gi) * 128, 128))
                for j in range(4):
                    row0 = b * D + (g0 + gi) * 128 + j * DH
                    accs, done = {}, 0

                    def vpu_piece(n, gate):
                        kg, part = n // VSPLIT, n % VSPLIT
                        for d in range(part * DH // VSPLIT, (part + 1) * DH // VSPLIT):
                            qrow = qf[pl.ds(row0 + d, 1), :]
                            for g in range(kg * VG, (kg + 1) * VG):
                                kcol = kb_ref[d, g * 8:(g + 1) * 8, :]
                                first_d = d == part * DH // VSPLIT
                                if gate is not None and (VGATE == 2 or first_d):
                                    kcol = pltpu.bitcast(pltpu.bitcast(kcol, U32) | gate, F32)
                                term = jnp.concatenate([kcol] * (CB // 128), axis=1) * qrow
                                accs[g] = term if d == 0 else accs[g] + term

                    for c, (kb, ks) in enumerate(chunks):
                        last = c == len(chunks) - 1
                        s = _dot(kp.get(j * NB + kb, rows=(ks.start, KC - NV_KEYS * last)), q)
                        if last:
                            s = jnp.concatenate([s] + [accs[g] for g in sorted(accs)], axis=0)
                        else:
                            upto = (c + 1) * n_pieces // (len(chunks) - 1)
                            for n in range(done, upto):
                                r = (n - done) * KC // (upto - done)
                                vpu_piece(n, pltpu.bitcast(s[r:r + 8, 0:128], U32) & zero if VGATE else None)
                            done = upto
                        pending.append((gi, j, c, s))
                        left = 4 * GPI * len(chunks) - 1 - ((gi * 4 + j) * len(chunks) + c)
                        if len(pending) > LAG and left >= HOLD:
                            pv(*pending.pop(0))
            for item in pending:
                pv(*item)
            return tot, lmin

        tot, lmin = lax.fori_loop(0, n_iter, attend,
                                  (jnp.zeros((8, CB), F32), jnp.ones((1, CB), F32)))

        safe = (tot <= 2.0 ** 120) & (lmin >= 2.0 ** -30)
        n_unsafe = jnp.sum(jnp.where(safe, 0.0, 1.0))

        @pl.when(n_unsafe > 0.0)
        def _():
            def attend_true_max(i, carry):
                b = i // (4 * NG)
                h = i % (4 * NG)
                q = qt.get(b, rows=((h // 4) * 128, 128))
                for c, (kb, ks) in enumerate(chunks):
                    sbuf[_tile(c, KC), :] = _dot(kp.get(h % 4 * NB + kb, rows=(ks.start, KC)), q)
                m = jnp.max(sbuf[...], axis=0, keepdims=True)
                acc = jnp.zeros((DH, CB), F32)
                l = jnp.zeros((8, CB), F32)
                for c, (kb, ks) in enumerate(chunks):
                    p = jnp.exp2(sbuf[_tile(c, KC), :] - m)
                    acc = acc + _dot(vt.get(kb, cols=ks), p.astype(BF16))
                    l = l + _fold8(p)
                ot[b, pl.ds(pl.multiple_of(h * DH, DH), DH), :] = acc / jnp.sum(l, axis=0, keepdims=True)
                return carry
            lax.fori_loop(0, NB * 4 * NG, attend_true_max, 0)

        def a_out(par, carry):
            out_proj(wot, par)
            return carry
        lax.fori_loop(0, 2, a_out, 0)

    def qkv_proj(g, par, first=False, marks=None):
        if first:
            right = _right_forms(normed(2 * par), normed(2 * par + 1))
            for i, form in enumerate(right):
                xn.put(form, 7 * par + i)
        else:
            right = [xn.get(7 * par + i) for i in range(7)]
        for half, r in enumerate(_strassen(lambda i: wqkvt.get(7 * g + i), right, marks, MPD, False)):
            qkv[par][:, _tile(half, CB)] = r

    def window(pair, g, par, marks=None, span=SPAN):
        buf = qkv[par]
        zero = jnp.full((8, 128), pair // 4096, jnp.int32).astype(U32)
        first = lax.broadcasted_iota(jnp.int32, (128, 128), 1) == 0
        even = lax.broadcasted_iota(jnp.int32, (8, 128), 0) % 2 == 0

        def paced(x, step):
            return gated(x, marks, span * step, zero)

        def tile(kind, u):
            return jnp.concatenate([buf[r:r + 64, _tile(u)] for r in (kind * 64, 192 + kind * 64)])

        k = [tile(1, t) for t in range(8)]
        v = [tile(2, t) for t in range(8)]
        v_first = jnp.broadcast_to(v[0][:, 0:1], (128, 128))
        ks = [None] + [pltpu.roll(x, 1, 1) for x in k[1:]]
        vs = [None] + [jnp.where(first, v_first, pltpu.roll(x, 1, 1)) for x in v[1:]]
        if GR:
            ks = [None] + [pltpu.roll(paced(x, (t - 1) / 8), 1, 1) for t, x in enumerate(k) if t]
        for u in range(8):
            q = tile(0, u).reshape(16, 8, 128)
            logits = []
            for t in range(8):
                if t % (8 // NQ) == 0:
                    scale = paced(jnp.full((8, 128), QK_SCALE, F32), (u + 0.5 * t / 8) / 8)
                    qs = q * scale
                lg = jnp.sum(qs * (k[t] if t <= u else ks[t]).reshape(16, 8, 128), axis=0)
                lg = lg + jnp.where(even, pltpu.roll(lg, 7, 0), pltpu.roll(lg, 1, 0))
                if t > u:
                    lg = jnp.where(first[0:8], -1e9 * LOG2E, lg)
                logits.append(lg)
            m = _tree(jnp.maximum, logits)
            p = [jnp.exp2(lg - m) for lg in logits]
            inv = pltpu.reciprocal(_tree(jnp.add, p), full_range=False)
            n = 16 // NV
            for part in range(NV):
                r = paced(inv, (u + 0.5 + 0.5 * part / NV) / 8)
                o = None
                for t in range(8):
                    x = (v[t] if t <= u else vs[t]).reshape(16, 8, 128)[part * n:(part + 1) * n]
                    pv = (p[t] * r) * x
                    o = pv if o is None else o + pv
                rows = pl.ds(pl.multiple_of(g * 128 + part * n * 8, n * 8), n * 8)
                ot[2 * par + u // 4, rows, _tile(u % 4)] = o.reshape(n * 8, 128)

    def layer_b(pair):
        qkv_proj(0, 0, first=True)
        marks = []
        qkv_proj(0, 1, first=True, marks=marks)
        window(pair, 0, 0, marks)

        def b_mix(g, carry):
            m0, m1 = [], []
            qkv_proj(g, 0, marks=m0)
            window(pair, g - 1, 1, m0)
            qkv_proj(g, 1, marks=m1)
            window(pair, g, 0, m1)
            return carry
        lax.fori_loop(1, NG, b_mix, 0)
        marks = []
        out_proj(wobt, 0, marks)
        window(pair, NG - 1, 1, marks, SPAN_W)

        zero = jnp.full((8, 128), pair // 4096, jnp.int32).astype(U32)
        for n, (kt, t) in enumerate((kt, t) for kt in range(4) for t in range(4)):
            frac = SPAN_F * n / 12 if kt < 3 else SPAN_L + (n - 12) * DL
            xs_ = [jnp.concatenate([gated(ot[b, _tile(k), _tile(t)], marks, frac, zero)
                                    for k in (kt, kt + 4)]) for b in (2, 3)]
            for i, form in enumerate(_right_forms(*xs_)):
                xn.put(form, i, rows=_rows(kt), cols=_tile(t))

        def b_out(i, carry):
            right = [xn.get(f) for f in range(7)]
            strips = [i * SPI + c for c in range(SPI)]
            for c in strips:
                rows = pl.ds(pl.multiple_of(c * 128, 128), 128)
                ys = _strassen(functools.partial(wobt.get, rows=_rows(c, 64)), right)
                for half, y in enumerate(ys):
                    b = 2 + half
                    x = xt[b, rows, :] + y
                    xt[b, rows, :] = x
                    pivot = jnp.where(c == 0, x[0:1], stats[b, 2, 0:1])
                    s1, s2 = shifted_sums(x, pivot)
                    stats[b, 0] = jnp.where(c == 0, 0.0, stats[b, 0]) + s1
                    stats[b, 1] = jnp.where(c == 0, 0.0, stats[b, 1]) + s2
                    stats[b, 2] = jnp.broadcast_to(pivot, (8, CB))
                    words = (as_bf16_bits(xt[half, rows, :]) >> 16) | as_bf16_bits(x)
                    for t in range(4):
                        xs_words[c, pl.ds(4 * half + t, 128, stride=8), :] = words[:, _tile(t)].T

            @pl.when(pair == 1)
            def _():
                for c in strips:
                    o_cp(c).start()
            return carry
        lax.fori_loop(0, 8 // SPI, b_out, 0)
        for b in (2, 3):
            put_stats(b, slice(None), stats[b, 2, 0:1], stats[b, 0], stats[b, 1])

        @pl.when(pair == 1)
        def _():
            for c in range(8):
                o_cp(c).wait()

    def as_bf16_bits(x):
        return pltpu.bitcast(x.astype(BF16).astype(F32), U32)

    def pair_body(pair, carry):
        layer_a(pair)
        layer_b(pair)
        return carry
    lax.fori_loop(0, 2, pair_body, 0)


@jax.jit
def pallas_interleave_layers__grouped_kv_mqa__sliding_local_dilated__prompt_kernel(
    A_x: jax.Array,
    A_wq: jax.Array,
    A_wk: jax.Array,
    A_wv: jax.Array,
    A_wo: jax.Array,
    B_x: jax.Array,
    B_wqkv: jax.Array,
    B_wo: jax.Array,
):
    del B_x
    hbm = pl.BlockSpec(memory_space=pl.ANY)
    vmem = pl.BlockSpec(memory_space=pltpu.VMEM)
    out = pl.pallas_call(
        _kernel,
        in_specs=[hbm, hbm, vmem, vmem, hbm, hbm, hbm],
        out_specs=hbm,
        out_shape=jax.ShapeDtypeStruct((S, D), BF16),
        scratch_shapes=[
            pltpu.VMEM((8, S, 128), BF16),
            pltpu.VMEM((D, D), BF16),
            pltpu.VMEM((D, D), BF16),
            pltpu.VMEM((D, 3 * D), BF16),
            pltpu.VMEM((D, D), BF16),
            pltpu.VMEM((DH, D), U32),
            pltpu.VMEM((7 * D // 4, D // 2), U32),
            pltpu.VMEM((7 * D // 4, D // 2), U32),
            pltpu.VMEM((NG * 7 * 96, D // 2), U32),
            pltpu.VMEM((7 * D // 4, D // 2), U32),
            pltpu.VMEM((NB, D, CB), F32),
            pltpu.VMEM((NB, 3, 8, CB), F32),
            pltpu.VMEM((2 * 7 * D // 4, CB), U32),
            pltpu.VMEM((NB * D // 2, CB), U32),
            pltpu.VMEM((NB * D, CB), F32),
            pltpu.VMEM((DH, NV_KEYS, 128), F32),
            pltpu.VMEM((NB, D, CB), F32),
            pltpu.VMEM((4 * S // 2, 128), U32),
            pltpu.VMEM((NB * DH // 2, CB), U32),
            pltpu.VMEM((S, CB), F32),
            pltpu.VMEM((384, 2 * CB), F32),
            pltpu.VMEM((384, 2 * CB), F32),
            pltpu.SemaphoreType.DMA((12,)),
        ],
        compiler_params=pltpu.CompilerParams(vmem_limit_bytes=110 * 1024 * 1024),
        name="interleave_stack",
    )(A_x.reshape(S, D), A_wq, A_wk.T, A_wv.T, A_wo, B_wqkv, B_wo)
    return out.reshape(1, S, D)
```

```python
import functools
import math

import jax
import jax.numpy as jnp
from jax import lax
import jax.experimental.pallas as pl
import jax.experimental.pallas.tpu as pltpu

S = 2048
D = 1024
DH = 32
NB = 4
CB = S // NB
NG = 8
EPS = 1e-5
LOG2E = math.log2(math.e)
QK_SCALE = DH ** -0.5 * LOG2E
KC = 256
GPI = 2
LAG = 1
MPD = 4
NSP = 5
NSQ = 7
NV_KEYS = 64
VG = 1
VSPLIT = 4
VGATE = 1
DL = 0.05
LW = 4
PSPLIT = 0
MPO = 8
SPAN_W = 0.75
SPAN_F = 0.85
SPAN_L = 0.8
SPAN = 0.9
NQ = 4
NV = 4
GR = 0
W0 = 1
GATE = 40
DELAY = 2
XF = 1
HOLD = 2
SPI = 2
F32 = jnp.float32
BF16 = jnp.bfloat16
U32 = jnp.uint32


def _dot(a, b):
    return jnp.dot(a, b, preferred_element_type=F32)


def _fold8(x):
    return jnp.sum(x.reshape(x.shape[0] // 8, 8, x.shape[1]), axis=0)


def _tree(op, xs):
    xs = list(xs)
    while len(xs) > 1:
        xs = [op(xs[i], xs[i + 1]) for i in range(0, len(xs), 2)]
    return xs[0]


def _tile(i, n=128):
    return slice(i * n, (i + 1) * n)


def _left_forms(a11, a12, a21, a22):
    return (a11 + a22, a21 + a22, a11, a22, a11 + a12, a21 - a11, a12 - a22)


def _heads_on_sublanes(x):
    x = x.reshape(8, 2, 8, x.shape[1])
    return [x[:, j].swapaxes(0, 1).reshape(64, x.shape[-1]) for j in range(2)]


def _right_forms(x0, x1):
    n = x0.shape[0] // 2
    b11, b21, b12, b22 = x0[:n], x0[n:], x1[:n], x1[n:]
    forms = (b11 + b22, b11, b12 - b22, b21 - b11, b22, b11 + b12, b21 + b22)
    return [f.astype(BF16) for f in forms]


def _strassen(left, right, marks=None, per_dot=2, n_split=7):
    def product(i, position):
        if marks is None or position >= n_split:
            return _dot(left(i), right[i])
        a, acc = left(i), None
        for kt in range(4):
            part = _dot(a[:, _tile(kt)], right[i][_tile(kt), :])
            marks.extend(part[m:m + 8, 0:128] for m in range(0, a.shape[0], a.shape[0] // per_dot))
            acc = part if acc is None else acc + part
        return acc
    m2, m4, m3, m5, m1, m7, m6 = (product(i - 1, n) for n, i in enumerate((2, 4, 3, 5, 1, 7, 6)))
    return [(1, 0, m2 + m4), (0, 1, m3 + m5), (0, 0, m4 - m5 + m1 + m7), (1, 1, m3 - m2 + m1 + m6)]


def _head_halves(y, row_half):
    return [(32 * n + 16 * row_half, y[16 * n:16 * (n + 1)]) for n in range(y.shape[0] // 16)]


class _Packed:
    def __init__(self, ref, n_rows):
        self.ref = ref
        self.n_rows = n_rows

    def _index(self, matrix, rows, cols):
        start, size = (0, self.n_rows) if rows is None else rows
        start = (matrix * self.n_rows + start) // 2
        if not isinstance(start, int):
            start = pl.multiple_of(start, 8)
        return pl.ds(start, size // 2), cols

    def get(self, matrix=0, rows=None, cols=slice(None)):
        return pltpu.bitcast(self.ref[self._index(matrix, rows, cols)], BF16)

    def put(self, value, matrix=0, rows=None, cols=slice(None)):
        self.ref[self._index(matrix, rows, cols)] = pltpu.bitcast(value.astype(BF16), U32)


def _rows(i, n=128):
    return i * n, n


def _kernel(x_hbm, wq_hbm, wkt_ref, wvt_ref, wo_hbm, wqkv_hbm, wob_hbm, out_hbm,
            xs, wq_s, wo_s, wqkv_s, wob_s, wkvt, wqt, wot, wqkvt, wobt,
            xt, stats, xn, qt, qf, ot, kp, vt, sbuf, qkv0, qkv1, sems):
    wkvt, wqkvt, qt = _Packed(wkvt, 2 * DH), _Packed(wqkvt, 192), _Packed(qt, D)
    wqt, wot, wobt, xn, kp = (_Packed(r, CB) for r in (wqt, wot, wobt, xn, kp))
    vt = _Packed(vt, DH)
    qkv = (qkv0, qkv1)

    def x_cp(c):
        c0 = c * 128 if isinstance(c, int) else pl.multiple_of(c * 128, 128)
        return pltpu.make_async_copy(x_hbm.at[:, pl.ds(c0, 128)], xs.at[c], sems.at[c])


    def o_cp(c):
        c0 = c * 128 if isinstance(c, int) else pl.multiple_of(c * 128, 128)
        return pltpu.make_async_copy(xs.at[c], out_hbm.at[:, pl.ds(c0, 128)], sems.at[c])

    w_cp = [pltpu.make_async_copy(src, dst, sems.at[8 + i]) for i, (src, dst) in enumerate(
        [(wq_hbm, wq_s), (wo_hbm, wo_s), (wqkv_hbm, wqkv_s), (wob_hbm, wob_s)])]
    xs_words = xs.bitcast(U32)

    def shifted_sums(x, pivot):
        d = x - pivot
        n = d.shape[0] // LW
        parts = [d[i * n:(i + 1) * n] for i in range(LW)]
        return _tree(jnp.add, map(_fold8, parts)), _tree(jnp.add, [_fold8(y * y) for y in parts])

    def put_stats(b, cols, pivot, s1, s2):
        s1 = jnp.sum(s1, axis=0, keepdims=True) * (1.0 / D)
        s2 = jnp.sum(s2, axis=0, keepdims=True) * (1.0 / D)
        rstd = lax.rsqrt(jnp.maximum(s2 - s1 * s1, 0.0) + EPS)
        stats[b, 0, :, cols] = jnp.broadcast_to(rstd, (8, rstd.shape[1]))
        stats[b, 1, :, cols] = jnp.broadcast_to((pivot + s1) * rstd, (8, rstd.shape[1]))

    def normed(b):
        return xt[b] * stats[b, 0, 0:1] - stats[b, 1, 0:1]

    def gated(x, marks, frac, zero):
        if marks is None:
            return x
        gate = pltpu.bitcast(marks[int(frac * len(marks))], U32) & zero
        x = jnp.broadcast_to(x, (max(8, x.shape[0]), 128))
        return pltpu.bitcast((pltpu.bitcast(x, U32).reshape(-1, 8, 128) | gate).reshape(-1, 128), F32)

    def out_proj(w, par, marks=None):
        ys = _strassen(w.get, _right_forms(ot[2 * par], ot[2 * par + 1]), marks, MPO, NSP)
        sums = {}
        for row_half, half, y in ys:
            b = 2 * par + half
            xs_ = []
            for r, piece in _head_halves(y, row_half):
                x = xt[b, r:r + 16, :] + piece
                xt[b, r:r + 16, :] = x
                xs_.append(x)
            if half not in sums:
                sums[half] = (xs_[0][0:1], *shifted_sums(jnp.concatenate(xs_), xs_[0][0:1]))
            else:
                pivot, s1, s2 = sums[half]
                t1, t2 = shifted_sums(jnp.concatenate(xs_), pivot)
                put_stats(b, slice(None), pivot, s1 + t1, s2 + t2)

    def prepare_steps(src, dst, base, row0, col0, kt):
        st = {}

        def load(half, gate=None):
            k0 = pl.multiple_of(kt * 128 + half * (D // 2), 128)
            t = src[pl.ds(k0, 128), pl.ds(pl.multiple_of(col0, 128), 128)]
            if gate is not None:
                w = pltpu.bitcast(t, U32).reshape(8, 8, 128) | gate
                t = pltpu.bitcast(w.reshape(64, 128), BF16)
            if src is wob_s:
                t = jnp.concatenate(_heads_on_sublanes(t.astype(F32)), axis=0).T
            else:
                t = t.T.astype(F32)
            st[half] = t

        def split(half, gate=None):
            t = st[half]
            if gate is not None and src is wqkv_s:
                w = pltpu.bitcast(t, U32).reshape(16, 8, 128) | gate
                t = pltpu.bitcast(w.reshape(128, 128), F32)
            if src is wqkv_s:
                st[half] = _heads_on_sublanes(t)
            else:
                t = t.reshape(4, 2, 16, 128)
                st[half] = (t[:, 0].reshape(64, 128), t[:, 1].reshape(64, 128))

        def store(gate=None):
            (a11, a21), (a12, a22) = st[0], st[1]
            for i, form in enumerate(_left_forms(a11, a12, a21, a22)):
                dst.put(form, base + i, rows=(row0, 64), cols=pl.ds(pl.multiple_of(kt * 128, 128), 128))

        P = functools.partial
        return [(0, P(load, 0)), (1, P(split, 0)), (1, P(load, 1)), (2, P(split, 1)), (2, store)]

    w_cp[0].start()
    for c in range(8):
        x_cp(c).start()
    wkvt.put(wkt_ref[...], rows=_rows(0, DH))
    wkvt.put(wvt_ref[...], rows=_rows(1, DH))
    stats[...] = jnp.zeros(stats.shape, F32)

    w_cp[0].wait()

    def transpose_wq(c, carry):
        for kt in range(4):
            for _, step in prepare_steps(wq_s, wqt, 0, c * 64, c * 128, kt):
                step()
        return carry
    lax.fori_loop(0, 8, transpose_wq, 0)

    def load_strip(c, carry):
        x_cp(c).wait()
        rows = pl.ds(pl.multiple_of(c * 128, 128), 128)
        for u in range(8):
            t = xs_words[c, pl.ds(u, 128, stride=8), :].T
            halves = (pltpu.bitcast(t << 16, F32), pltpu.bitcast(t & U32(0xFFFF0000), F32))
            for par, x in enumerate(halves):
                b, cols = 2 * par + u // 4, _tile(u % 4)
                xt[b, rows, cols] = x
                pivot = jnp.where(c == 0, x[0:1], stats[b, 2, :, cols])
                s1, s2 = shifted_sums(x, pivot[0:1])
                stats[b, 0, :, cols] += s1
                stats[b, 1, :, cols] += s2
                stats[b, 2, :, cols] = pivot
        return carry
    lax.fori_loop(0, 8, load_strip, 0)
    for cp in w_cp[1:]:
        cp.start()
    for b in range(NB):
        put_stats(b, slice(None), stats[b, 2], stats[b, 0], stats[b, 1])

    def other_weights(i, n):
        units = []
        for u in range(32 // n):
            c, kt = (i * (32 // n) + u) // 4, (i * (32 // n) + u) % 4
            units.append((wo_s, wot, 0, c * 64, c * 128, kt))
            units.append((wob_s, wobt, 0, c * 64, c * 128, kt))
            units += [(wqkv_s, wqkvt, 7 * c, j * 64, j * D + c * 128, kt) for j in range(3)]
        return units

    def key_rows(i, start, size):
        return pl.ds(NB * D + i * NV_KEYS + start, size)

    def layer_a(pair):
        lane_head = lax.broadcasted_iota(jnp.int32, (64, 128), 1) // DH

        def project(par, shift):
            xs_ = [normed(2 * par + half) for half in range(2)]
            kvs = [_dot(wkvt.get(), x.astype(BF16)) for x in xs_]
            shift = jnp.where(par == 0, jnp.mean(kvs[0][0:DH], axis=1, keepdims=True), shift)
            for half, kv in enumerate(kvs):
                b = 2 * par + half
                k = (kv[0:DH] - shift) * QK_SCALE
                vt.put(kv[DH:], b)
                for t in range(CB // 128):
                    krep = jnp.concatenate([k[:, _tile(t)]] * 4, axis=0).T
                    words = pltpu.bitcast(krep.astype(BF16), U32)
                    if half == 1 and t == CB // 128 - 1:
                        for d in range(DH):
                            qf[key_rows(d // 4, 0, NV_KEYS), _tile(d % 4)] = jnp.broadcast_to(
                                krep[128 - NV_KEYS:, d:d + 1], (NV_KEYS, 128))
                    for j in range(4):
                        kp.ref[pl.ds(pl.multiple_of((j * NB + b) * (CB // 2) + t * 64, 64), 64), :] = (
                            jnp.where(lane_head == j, words, U32(0)))
            for row_half, half, q in _strassen(wqt.get, _right_forms(*xs_)):
                for r, piece in _head_halves(q, row_half):
                    qt.put(piece, 2 * par + half, rows=(r, 16))
                    qf[pl.ds(pl.multiple_of((2 * par + half) * D + r, 16), 16), :] = piece
            return shift
        lax.fori_loop(0, 2, project, jnp.zeros((DH, 1), F32))

        @pl.when(pair == 0)
        def _():
            for cp in w_cp[1:]:
                cp.wait()

        chunks = [(c // (CB // KC), _tile(c % (CB // KC), KC)) for c in range(S // KC)]
        n_iter = NB * NG // GPI

        def attend(i, carry):
            tot, lmin = carry
            b = i // (NG // GPI)
            g0 = (i % (NG // GPI)) * GPI
            state = {}
            units = other_weights(i, n_iter)
            zero = jnp.full((8, 128), i // 4096, jnp.int32).astype(U32)
            steps = [((u * GATE) // len(units) + d * DELAY, step)
                     for u, unit in enumerate(units) for d, step in prepare_steps(*unit)]

            def pv(gi, j, c, s):
                nonlocal tot, lmin
                kb, ks = chunks[c]
                p = jnp.exp2(s)
                for spot, step in steps:
                    if spot == (gi * 4 + j) * len(chunks) + c:
                        step(pltpu.bitcast(p[0:8, 0:128], U32) & zero)
                acc = _dot(vt.get(kb, cols=ks), p.astype(BF16))
                l = _fold8(p)
                if c > 0:
                    acc = acc + state[gi, j][0]
                    l = l + state[gi, j][1]
                state[gi, j] = (acc, l)
                if c == len(chunks) - 1:
                    l = jnp.sum(l, axis=0, keepdims=True)
                    tot = tot + (_fold8(jnp.abs(acc)) + l)
                    lmin = jnp.minimum(lmin, l)
                    row = pl.multiple_of((g0 + gi) * 128 + j * DH, DH)
                    ot[b, pl.ds(row, DH), :] = acc * pltpu.reciprocal(l, full_range=False)

            pending = []
            n_pieces = NV_KEYS // (8 * VG) * VSPLIT
            for gi in range(GPI):
                q = qt.get(b, rows=((g0 + gi) * 128, 128))
                for j in range(4):
                    row0 = b * D + (g0 + gi) * 128 + j * DH
                    accs, done = {}, 0

                    def vpu_piece(n, gate):
                        kg, part = n // VSPLIT, n % VSPLIT
                        for d in range(part * DH // VSPLIT, (part + 1) * DH // VSPLIT):
                            qrow = qf[pl.ds(row0 + d, 1), :]
                            for g in range(kg * VG, (kg + 1) * VG):
                                kcol = qf[key_rows(d // 4, g * 8, 8), _tile(d % 4)]
                                first_d = d == part * DH // VSPLIT
                                if gate is not None and (VGATE == 2 or first_d):
                                    kcol = pltpu.bitcast(pltpu.bitcast(kcol, U32) | gate, F32)
                                term = jnp.concatenate([kcol] * (CB // 128), axis=1) * qrow
                                accs[g] = term if d == 0 else accs[g] + term

                    for c, (kb, ks) in enumerate(chunks):
                        last = c == len(chunks) - 1
                        s = _dot(kp.get(j * NB + kb, rows=(ks.start, KC - NV_KEYS * last)), q)
                        if last:
                            s = jnp.concatenate([s] + [accs[g] for g in sorted(accs)], axis=0)
                        else:
                            upto = (c + 1) * n_pieces // (len(chunks) - 1)
                            for n in range(done, upto):
                                r = (n - done) * KC // (upto - done)
                                vpu_piece(n, pltpu.bitcast(s[r:r + 8, 0:128], U32) & zero if VGATE else None)
                            done = upto
                        pending.append((gi, j, c, s))
                        left = 4 * GPI * len(chunks) - 1 - ((gi * 4 + j) * len(chunks) + c)
                        if len(pending) > LAG and left >= HOLD:
                            pv(*pending.pop(0))
            for item in pending:
                pv(*item)
            return tot, lmin

        tot, lmin = lax.fori_loop(0, n_iter, attend,
                                  (jnp.zeros((8, CB), F32), jnp.ones((1, CB), F32)))

        safe = (tot <= 2.0 ** 120) & (lmin >= 2.0 ** -30)
        n_unsafe = jnp.sum(jnp.where(safe, 0.0, 1.0))

        @pl.when(n_unsafe > 0.0)
        def _():
            def attend_true_max(i, carry):
                b = i // (4 * NG)
                h = i % (4 * NG)
                q = qt.get(b, rows=((h // 4) * 128, 128))
                for c, (kb, ks) in enumerate(chunks):
                    sbuf[_tile(c, KC), :] = _dot(kp.get(h % 4 * NB + kb, rows=(ks.start, KC)), q)
                m = jnp.max(sbuf[...], axis=0, keepdims=True)
                acc = jnp.zeros((DH, CB), F32)
                l = jnp.zeros((8, CB), F32)
                for c, (kb, ks) in enumerate(chunks):
                    p = jnp.exp2(sbuf[_tile(c, KC), :] - m)
                    acc = acc + _dot(vt.get(kb, cols=ks), p.astype(BF16))
                    l = l + _fold8(p)
                ot[b, pl.ds(pl.multiple_of(h * DH, DH), DH), :] = acc / jnp.sum(l, axis=0, keepdims=True)
                return carry
            lax.fori_loop(0, NB * 4 * NG, attend_true_max, 0)

        def a_out(par, carry):
            out_proj(wot, par)
            return carry
        lax.fori_loop(0, 2, a_out, 0)

    def qkv_proj(g, par, first=False, marks=None):
        if first:
            right = _right_forms(normed(2 * par), normed(2 * par + 1))
            for i, form in enumerate(right):
                xn.put(form, 7 * par + i)
        else:
            right = [xn.get(7 * par + i) for i in range(7)]
        ys = _strassen(lambda i: wqkvt.get(7 * g + i), right, marks, MPD, NSQ)
        for row_half, half, y in ys:
            qkv[par][_tile(row_half, 192), _tile(half, CB)] = y

    def window(pair, g, par, marks=None, span=SPAN):
        buf = qkv[par]
        zero = jnp.full((8, 128), pair // 4096, jnp.int32).astype(U32)
        first = lax.broadcasted_iota(jnp.int32, (128, 128), 1) == 0
        even = lax.broadcasted_iota(jnp.int32, (8, 128), 0) % 2 == 0

        def paced(x, step):
            return gated(x, marks, span * step, zero)

        def tile(kind, u):
            return jnp.concatenate([buf[r:r + 64, _tile(u)] for r in (kind * 64, 192 + kind * 64)])

        k = [tile(1, t) for t in range(8)]
        v = [tile(2, t) for t in range(8)]
        v_first = jnp.broadcast_to(v[0][:, 0:1], (128, 128))
        ks = [None] + [pltpu.roll(x, 1, 1) for x in k[1:]]
        vs = [None] + [jnp.where(first, v_first, pltpu.roll(x, 1, 1)) for x in v[1:]]
        if GR:
            ks = [None] + [pltpu.roll(paced(x, (t - 1) / 8), 1, 1) for t, x in enumerate(k) if t]
        for u in range(8):
            q = tile(0, u).reshape(16, 8, 128)
            logits = []
            for t in range(8):
                if t % (8 // NQ) == 0:
                    scale = paced(jnp.full((8, 128), QK_SCALE, F32), (u + 0.5 * t / 8) / 8)
                    qs = q * scale
                lg = jnp.sum(qs * (k[t] if t <= u else ks[t]).reshape(16, 8, 128), axis=0)
                lg = lg + jnp.where(even, pltpu.roll(lg, 7, 0), pltpu.roll(lg, 1, 0))
                if t > u:
                    lg = jnp.where(first[0:8], -1e9 * LOG2E, lg)
                logits.append(lg)
            m = _tree(jnp.maximum, logits)
            p = [jnp.exp2(lg - m) for lg in logits]
            inv = pltpu.reciprocal(_tree(jnp.add, p), full_range=False)
            n = 16 // NV
            for part in range(NV):
                r = paced(inv, (u + 0.5 + 0.5 * part / NV) / 8)
                o = None
                for t in range(8):
                    x = (v[t] if t <= u else vs[t]).reshape(16, 8, 128)[part * n:(part + 1) * n]
                    pv = (p[t] * r) * x
                    o = pv if o is None else o + pv
                rows = pl.ds(pl.multiple_of(g * 128 + part * n * 8, n * 8), n * 8)
                ot[2 * par + u // 4, rows, _tile(u % 4)] = o.reshape(n * 8, 128)

    def layer_b(pair):
        qkv_proj(0, 0, first=True)
        marks = []
        qkv_proj(0, 1, first=True, marks=marks)
        window(pair, 0, 0, marks)

        def b_mix(g, carry):
            m0, m1 = [], []
            qkv_proj(g, 0, marks=m0)
            window(pair, g - 1, 1, m0)
            qkv_proj(g, 1, marks=m1)
            window(pair, g, 0, m1)
            return carry
        lax.fori_loop(1, NG, b_mix, 0)
        marks = []
        out_proj(wobt, 0, marks)
        window(pair, NG - 1, 1, marks, SPAN_W)

        zero = jnp.full((8, 128), pair // 4096, jnp.int32).astype(U32)
        for n, (kt, t) in enumerate((kt, t) for kt in range(4) for t in range(4)):
            frac = SPAN_F * n / 12 if kt < 3 else SPAN_L + (n - 12) * DL
            xs_ = [jnp.concatenate([gated(ot[b, _tile(k), _tile(t)], marks, frac, zero)
                                    for k in (kt, kt + 4)]) for b in (2, 3)]
            for i, form in enumerate(_right_forms(*xs_)):
                xn.put(form, i, rows=_rows(kt), cols=_tile(t))

        def b_out(i, carry):
            right = [xn.get(f) for f in range(7)]
            row0 = pl.multiple_of(i * SPI * 128, SPI * 128)
            ys = _strassen(functools.partial(wobt.get, rows=_rows(i, SPI * 64)), right)
            for half in range(2):
                b = 2 + half
                y = jnp.concatenate([piece for _, piece in sorted(
                    (p for rh, h, q in ys if h == half for p in _head_halves(q, rh)),
                    key=lambda p: p[0])])
                x = xt[b, pl.ds(row0, SPI * 128), :] + y
                xt[b, pl.ds(row0, SPI * 128), :] = x
                pivot = jnp.where(i == 0, x[0:1], stats[b, 2, 0:1])
                s1, s2 = shifted_sums(x, pivot)
                stats[b, 0] = jnp.where(i == 0, 0.0, stats[b, 0]) + s1
                stats[b, 1] = jnp.where(i == 0, 0.0, stats[b, 1]) + s2
                stats[b, 2] = jnp.broadcast_to(pivot, (8, CB))
                even = xt[half, pl.ds(row0, SPI * 128), :]
                words = (as_bf16_bits(even) >> 16) | as_bf16_bits(x)
                for c in range(SPI):
                    for t in range(4):
                        xs_words[i * SPI + c, pl.ds(4 * half + t, 128, stride=8), :] = (
                            words[_tile(c), _tile(t)].T)

            @pl.when(pair == 1)
            def _():
                for c in range(SPI):
                    o_cp(i * SPI + c).start()
            return carry
        lax.fori_loop(0, 8 // SPI, b_out, 0)
        for b in (2, 3):
            put_stats(b, slice(None), stats[b, 2, 0:1], stats[b, 0], stats[b, 1])

        @pl.when(pair == 1)
        def _():
            for c in range(8):
                o_cp(c).wait()

    def as_bf16_bits(x):
        return pltpu.bitcast(x.astype(BF16).astype(F32), U32)

    def pair_body(pair, carry):
        layer_a(pair)
        layer_b(pair)
        return carry
    lax.fori_loop(0, 2, pair_body, 0)


@jax.jit
def pallas_interleave_layers__grouped_kv_mqa__sliding_local_dilated__prompt_kernel(
    A_x: jax.Array,
    A_wq: jax.Array,
    A_wk: jax.Array,
    A_wv: jax.Array,
    A_wo: jax.Array,
    B_x: jax.Array,
    B_wqkv: jax.Array,
    B_wo: jax.Array,
):
    del B_x
    hbm = pl.BlockSpec(memory_space=pl.ANY)
    vmem = pl.BlockSpec(memory_space=pltpu.VMEM)
    out = pl.pallas_call(
        _kernel,
        in_specs=[hbm, hbm, vmem, vmem, hbm, hbm, hbm],
        out_specs=hbm,
        out_shape=jax.ShapeDtypeStruct((S, D), BF16),
        scratch_shapes=[
            pltpu.VMEM((8, S, 128), BF16),
            pltpu.VMEM((D, D), BF16),
            pltpu.VMEM((D, D), BF16),
            pltpu.VMEM((D, 3 * D), BF16),
            pltpu.VMEM((D, D), BF16),
            pltpu.VMEM((DH, D), U32),
            pltpu.VMEM((7 * D // 4, D // 2), U32),
            pltpu.VMEM((7 * D // 4, D // 2), U32),
            pltpu.VMEM((NG * 7 * 96, D // 2), U32),
            pltpu.VMEM((7 * D // 4, D // 2), U32),
            pltpu.VMEM((NB, D, CB), F32),
            pltpu.VMEM((NB, 3, 8, CB), F32),
            pltpu.VMEM((2 * 7 * D // 4, CB), U32),
            pltpu.VMEM((NB * D // 2, CB), U32),
            pltpu.VMEM((NB * D + DH * NV_KEYS // 4, CB), F32),
            pltpu.VMEM((NB, D, CB), F32),
            pltpu.VMEM((4 * S // 2, 128), U32),
            pltpu.VMEM((NB * DH // 2, CB), U32),
            pltpu.VMEM((S, CB), F32),
            pltpu.VMEM((384, 2 * CB), F32),
            pltpu.VMEM((384, 2 * CB), F32),
            pltpu.SemaphoreType.DMA((12,)),
        ],
        compiler_params=pltpu.CompilerParams(vmem_limit_bytes=110 * 1024 * 1024),
        name="interleave_stack",
    )(A_x.reshape(S, D), A_wq, A_wk.T, A_wv.T, A_wo, B_wqkv, B_wo)
    return out.reshape(1, S, D)
```

```python
import functools
import math

import numpy as np

import jax
import jax.numpy as jnp
from jax import lax
import jax.experimental.pallas as pl
import jax.experimental.pallas.tpu as pltpu

S = 2048
D = 1024
DH = 32
NB = 4
CB = S // NB
NG = 8
EPS = 1e-5
LOG2E = math.log2(math.e)
QK_SCALE = DH ** -0.5 * LOG2E
MASKED = -1e9 * LOG2E

KC = 256
GPI = 2
VPU_KEYS = 64
VPU_SPLIT = 8
OUT_STRIPS = 2

F32 = jnp.float32
BF16 = jnp.bfloat16
U32 = jnp.uint32


def _dot(a, b):
    return jnp.dot(a, b, preferred_element_type=F32)


def _fold8(x):
    return jnp.sum(x.reshape(x.shape[0] // 8, 8, x.shape[1]), axis=0)


def _tree(op, xs):
    xs = list(xs)
    while len(xs) > 1:
        xs = [op(xs[i], xs[i + 1]) for i in range(0, len(xs), 2)]
    return xs[0]


def _tile(i, n=128):
    return slice(i * n, (i + 1) * n)


def _ds(start, size, align):
    return pl.ds(start if isinstance(start, int) else pl.multiple_of(start, align), size)


def _zero_bits(counter):
    return jnp.full((8, 128), counter // 4096, jnp.int32).astype(U32)


def _gate(x, zeros):
    words = pltpu.bitcast(x, U32)
    gated = words.reshape(-1, 8, 128) | zeros
    return pltpu.bitcast(gated.reshape(words.shape), x.dtype)


def _gate_at(x, marks, fraction, zero):
    return _gate(x, pltpu.bitcast(marks[int(fraction * len(marks))], U32) & zero)


def _heads_on_sublanes(x):
    x = x.reshape(8, 2, 8, x.shape[1])
    return [x[:, j].swapaxes(0, 1).reshape(64, x.shape[-1]) for j in range(2)]


def _left_forms(a11, a12, a21, a22):
    return (a11 + a22, a21 + a22, a11, a22, a11 + a12, a21 - a11, a12 - a22)


def _right_forms(x0, x1):
    n = x0.shape[0] // 2
    b11, b21, b12, b22 = x0[:n], x0[n:], x1[:n], x1[n:]
    forms = (b11 + b22, b11, b12 - b22, b21 - b11, b22, b11 + b12, b21 + b22)
    return [f.astype(BF16) for f in forms]


def _strassen(left, right, marks=None, marks_per_dot=0, marked_products=0):
    def product(i, position):
        if position >= marked_products:
            return _dot(left(i), right[i])
        a, acc = left(i), None
        for kt in range(4):
            part = _dot(a[:, _tile(kt)], right[i][_tile(kt), :])
            marks.extend(part[m:m + 8, 0:128]
                         for m in range(0, a.shape[0], a.shape[0] // marks_per_dot))
            acc = part if acc is None else acc + part
        return acc
    m2, m4, m3, m5, m1, m7, m6 = (
        product(i - 1, n) for n, i in enumerate((2, 4, 3, 5, 1, 7, 6)))
    return [(1, 0, m2 + m4), (0, 1, m3 + m5), (0, 0, m4 - m5 + m1 + m7), (1, 1, m3 - m2 + m1 + m6)]


def _head_halves(y, row_half):
    return [(32 * n + 16 * row_half, y[16 * n:16 * (n + 1)]) for n in range(y.shape[0] // 16)]


class _Packed:
    def __init__(self, ref, n_rows):
        self.ref = ref
        self.n_rows = n_rows

    def words(self, matrix, rows):
        start, size = (0, self.n_rows) if rows is None else rows
        return _ds((matrix * self.n_rows + start) // 2, size // 2, 8)

    def get(self, matrix=0, rows=None, cols=slice(None)):
        return pltpu.bitcast(self.ref[self.words(matrix, rows), cols], BF16)

    def put(self, value, matrix=0, rows=None, cols=slice(None)):
        self.ref[self.words(matrix, rows), cols] = pltpu.bitcast(value.astype(BF16), U32)


def _rows(i, n=128):
    return i * n, n


def _kernel(x_hbm, wq_hbm, wkt_ref, wvt_ref, wo_hbm, wqkv_hbm, wob_hbm, out_hbm,
            xs, wq_s, wo_s, wqkv_s, wob_s, wkvt, wqt, wot, wqkvt, wobt,
            xt, stats, xn, qt, qf, ot, kp, vt, sbuf, qkv0, qkv1, sems):
    wkvt, wqkvt = _Packed(wkvt, 2 * DH), _Packed(wqkvt, 192)
    wqt, wot, wobt, xn, kp = (_Packed(r, CB) for r in (wqt, wot, wobt, xn, kp))
    qt, vt = _Packed(qt, D), _Packed(vt, DH)
    qkv = (qkv0, qkv1)

    def x_cp(c):
        return pltpu.make_async_copy(
            x_hbm.at[:, _ds(c * 128, 128, 128)], xs.at[c, pl.ds(0, S)], sems.at[c])

    def out_cp(c):
        return pltpu.make_async_copy(
            xs.at[c, pl.ds(0, S)], out_hbm.at[:, _ds(c * 128, 128, 128)], sems.at[c])

    w_cp = [pltpu.make_async_copy(src, dst, sems.at[8 + i]) for i, (src, dst) in enumerate(
        [(wq_hbm, wq_s), (wo_hbm, wo_s), (wqkv_hbm, wqkv_s), (wob_hbm, wob_s)])]
    xs_words = xs.bitcast(U32)

    def shifted_sums(x, pivot):
        d = x - pivot
        n = d.shape[0] // 4
        parts = [d[_tile(i, n)] for i in range(4)]
        return _tree(jnp.add, map(_fold8, parts)), _tree(jnp.add, [_fold8(y * y) for y in parts])

    def put_stats(b, pivot, s1, s2):
        s1 = jnp.sum(s1, axis=0, keepdims=True) * (1.0 / D)
        s2 = jnp.sum(s2, axis=0, keepdims=True) * (1.0 / D)
        rstd = lax.rsqrt(jnp.maximum(s2 - s1 * s1, 0.0) + EPS)
        stats[b, 0] = jnp.broadcast_to(rstd, (8, CB))
        stats[b, 1] = jnp.broadcast_to((pivot + s1) * rstd, (8, CB))

    def normed(b):
        return xt[b] * stats[b, 0, 0:1] - stats[b, 1, 0:1]

    def out_proj(w, par, *marking):
        sums = {}
        for row_half, half, y in _strassen(
                w.get, _right_forms(ot[2 * par], ot[2 * par + 1]), *marking):
            b = 2 * par + half
            pieces = []
            for r, piece in _head_halves(y, row_half):
                x = xt[b, r:r + 16, :] + piece
                xt[b, r:r + 16, :] = x
                pieces.append(x)
            if half not in sums:
                pivot = pieces[0][0:1]
                sums[half] = (pivot, *shifted_sums(jnp.concatenate(pieces), pivot))
            else:
                pivot, s1, s2 = sums[half]
                t1, t2 = shifted_sums(jnp.concatenate(pieces), pivot)
                put_stats(b, pivot, s1 + t1, s2 + t2)

    def prepare_steps(src, dst, base, row0, col0, kt):
        st = {}

        def load(half, gate=None):
            t = src[_ds(kt * 128 + half * (D // 2), 128, 128), _ds(col0, 128, 128)]
            if gate is not None:
                t = _gate(t, gate)
            if src is wob_s:
                st[half] = jnp.concatenate(_heads_on_sublanes(t.astype(F32)), axis=0).T
            else:
                st[half] = t.T.astype(F32)

        def split(half, gate=None):
            t = st[half]
            if src is wqkv_s:
                st[half] = _heads_on_sublanes(t if gate is None else _gate(t, gate))
            else:
                t = t.reshape(4, 2, 16, 128)
                st[half] = (t[:, 0].reshape(64, 128), t[:, 1].reshape(64, 128))

        def store(gate=None):
            (a11, a21), (a12, a22) = st[0], st[1]
            for i, form in enumerate(_left_forms(a11, a12, a21, a22)):
                dst.put(form, base + i, rows=(row0, 64), cols=_ds(kt * 128, 128, 128))

        part = functools.partial
        return [(0, part(load, 0)), (2, part(split, 0)), (2, part(load, 1)),
                (4, part(split, 1)), (4, store)]

    def other_weights(i, n):
        units = []
        for u in range(32 // n):
            c, kt = (i * (32 // n) + u) // 4, (i * (32 // n) + u) % 4
            units.append((wo_s, wot, 0, c * 64, c * 128, kt))
            units.append((wob_s, wobt, 0, c * 64, c * 128, kt))
            units += [(wqkv_s, wqkvt, 7 * c, j * 64, j * D + c * 128, kt) for j in range(3)]
        return units

    w_cp[0].start()
    for c in range(8):
        x_cp(c).start()
    wkvt.put(wkt_ref[...], rows=_rows(0, DH))
    wkvt.put(wvt_ref[...], rows=_rows(1, DH))
    stats[...] = jnp.zeros(stats.shape, F32)
    w_cp[0].wait()

    def prepare_wq(c, carry):
        for kt in range(4):
            for _, step in prepare_steps(wq_s, wqt, 0, c * 64, c * 128, kt):
                step()
        return carry
    lax.fori_loop(0, 8, prepare_wq, 0)

    def load_strip(c, carry):
        x_cp(c).wait()
        for u in range(8):
            t = xs_words[c, pl.ds(u, 128, stride=8), :].T
            halves = (pltpu.bitcast(t << 16, F32),
                      pltpu.bitcast(t & np.uint32(0xFFFF0000), F32))
            for par, x in enumerate(halves):
                b, cols = 2 * par + u // 4, _tile(u % 4)
                xt[b, _ds(c * 128, 128, 128), cols] = x
                pivot = jnp.where(c == 0, x[0:1], stats[b, 2, :, cols])
                s1, s2 = shifted_sums(x, pivot[0:1])
                stats[b, 0, :, cols] += s1
                stats[b, 1, :, cols] += s2
                stats[b, 2, :, cols] = pivot
        return carry
    lax.fori_loop(0, 8, load_strip, 0)
    for cp in w_cp[1:]:
        cp.start()
    for b in range(NB):
        put_stats(b, stats[b, 2, 0:1], stats[b, 0], stats[b, 1])

    def key_column(d, start, size):
        return pl.ds(NB * D + d // 4 * VPU_KEYS + start, size), _tile(d % 4)

    def layer_a(pair):
        def project(par, shift):
            lane_head = lax.broadcasted_iota(jnp.int32, (64, 128), 1) // DH
            blocks = [normed(2 * par + half) for half in range(2)]
            kvs = [_dot(wkvt.get(), x.astype(BF16)) for x in blocks]
            shift = jnp.where(par == 0, jnp.mean(kvs[0][0:DH], axis=1, keepdims=True), shift)
            for half, kv in enumerate(kvs):
                b = 2 * par + half
                k = (kv[0:DH] - shift) * QK_SCALE
                vt.put(kv[DH:], b)
                for t in range(CB // 128):
                    krep = jnp.concatenate([k[:, _tile(t)]] * 4, axis=0).T
                    if half == 1 and t == CB // 128 - 1:
                        for d in range(DH):
                            qf[key_column(d, 0, VPU_KEYS)] = jnp.broadcast_to(
                                krep[128 - VPU_KEYS:, d:d + 1], (VPU_KEYS, 128))
                    words = pltpu.bitcast(krep.astype(BF16), U32)
                    for j in range(4):
                        kp.ref[kp.words(j * NB + b, _rows(t)), :] = jnp.where(
                            lane_head == j, words, np.uint32(0))
            for row_half, half, q in _strassen(wqt.get, _right_forms(*blocks)):
                for r, piece in _head_halves(q, row_half):
                    qt.put(piece, 2 * par + half, rows=(r, 16))
                    qf[_ds((2 * par + half) * D + r, 16, 16), :] = piece
            return shift
        lax.fori_loop(0, 2, project, jnp.zeros((DH, 1), F32))

        @pl.when(pair == 0)
        def _():
            for cp in w_cp[1:]:
                cp.wait()

        n_chunks = S // KC
        n_iter = NB * NG // GPI

        def chunk(c):
            return divmod(c * KC, CB)

        def attend(i, carry):
            total, lmin = carry
            b = i // (NG // GPI)
            g0 = (i % (NG // GPI)) * GPI
            zero = _zero_bits(i)
            units = other_weights(i, n_iter)
            steps = [((u * 40) // len(units) + delay, step)
                     for u, unit in enumerate(units) for delay, step in prepare_steps(*unit)]
            state = {}

            def accumulate(head, c, s):
                nonlocal total, lmin
                kb, k0 = chunk(c)
                p = jnp.exp2(s)
                for spot, step in steps:
                    if spot == head * n_chunks + c:
                        step(pltpu.bitcast(p[0:8, 0:128], U32) & zero)
                acc = _dot(vt.get(kb, cols=slice(k0, k0 + KC)), p.astype(BF16))
                l = _fold8(p)
                if c > 0:
                    acc = acc + state[head][0]
                    l = l + state[head][1]
                state[head] = (acc, l)
                if c == n_chunks - 1:
                    l = jnp.sum(l, axis=0, keepdims=True)
                    total = total + (_fold8(jnp.abs(acc)) + l)
                    lmin = jnp.minimum(lmin, l)
                    ot[b, _ds(g0 * 128 + head * DH, DH, DH), :] = (
                        acc * pltpu.reciprocal(l, full_range=False))

            def vpu_scores(head, n, gate, accs):
                group, part = divmod(n, VPU_SPLIT)
                ds = range(part * DH // VPU_SPLIT, (part + 1) * DH // VPU_SPLIT)
                for d in ds:
                    q_row = qf[pl.ds(b * D + g0 * 128 + head * DH + d, 1), :]
                    k_col = qf[key_column(d, group * 8, 8)]
                    if d == ds[0]:
                        k_col = _gate(k_col, gate)
                    term = jnp.concatenate([k_col] * (CB // 128), axis=1) * q_row
                    accs[group] = term if d == 0 else accs[group] + term

            pending = []
            n_pieces = VPU_KEYS // 8 * VPU_SPLIT
            left = 4 * GPI * n_chunks
            for head in range(4 * GPI):
                if head % 4 == 0:
                    q = qt.get(b, rows=(g0 * 128 + head * DH, 128))
                accs, done = {}, 0
                for c in range(n_chunks):
                    kb, k0 = chunk(c)
                    last = c == n_chunks - 1
                    s = _dot(kp.get(head % 4 * NB + kb, rows=(k0, KC - VPU_KEYS * last)), q)
                    if last:
                        s = jnp.concatenate([s] + [accs[g] for g in sorted(accs)], axis=0)
                    else:
                        upto = (c + 1) * n_pieces // (n_chunks - 1)
                        for n in range(done, upto):
                            r = (n - done) * KC // (upto - done)
                            vpu_scores(head, n, pltpu.bitcast(s[r:r + 8, 0:128], U32) & zero, accs)
                        done = upto
                    pending.append((head, c, s))
                    left -= 1
                    if len(pending) > 1 and left >= 2:
                        accumulate(*pending.pop(0))
            for item in pending:
                accumulate(*item)
            return total, lmin

        total, lmin = lax.fori_loop(
            0, n_iter, attend, (jnp.zeros((8, CB), F32), jnp.ones((1, CB), F32)))

        safe = (total <= 2.0 ** 120) & (lmin >= 2.0 ** -30)
        n_unsafe = jnp.sum(jnp.where(safe, 0.0, 1.0))

        @pl.when(n_unsafe > 0.0)
        def _():
            def attend_true_max(i, carry):
                b, h = i // (4 * NG), i % (4 * NG)
                q = qt.get(b, rows=_rows(h // 4))
                for c in range(n_chunks):
                    kb, k0 = chunk(c)
                    sbuf[_tile(c, KC), :] = _dot(kp.get(h % 4 * NB + kb, rows=(k0, KC)), q)
                m = jnp.max(sbuf[...], axis=0, keepdims=True)
                acc = jnp.zeros((DH, CB), F32)
                l = jnp.zeros((8, CB), F32)
                for c in range(n_chunks):
                    kb, k0 = chunk(c)
                    p = jnp.exp2(sbuf[_tile(c, KC), :] - m)
                    acc = acc + _dot(vt.get(kb, cols=slice(k0, k0 + KC)), p.astype(BF16))
                    l = l + _fold8(p)
                ot[b, _ds(h * DH, DH, DH), :] = acc / jnp.sum(l, axis=0, keepdims=True)
                return carry
            lax.fori_loop(0, NB * 4 * NG, attend_true_max, 0)

        def a_out(par, carry):
            out_proj(wot, par)
            return carry
        lax.fori_loop(0, 2, a_out, 0)

    def qkv_proj(g, par, marks=None, first=False):
        if first:
            right = _right_forms(normed(2 * par), normed(2 * par + 1))
            for i, form in enumerate(right):
                xn.put(form, 7 * par + i)
        else:
            right = [xn.get(7 * par + i) for i in range(7)]
        marking = () if marks is None else (marks, 4, 7)
        for row_half, half, y in _strassen(lambda i: wqkvt.get(7 * g + i), right, *marking):
            qkv[par][_tile(row_half, 192), _tile(half, CB)] = y

    def window(g, par, marks, zero, span):
        buf = qkv[par]
        first = lax.broadcasted_iota(jnp.int32, (128, 128), 1) == 0
        even = lax.broadcasted_iota(jnp.int32, (8, 128), 0) % 2 == 0

        def paced(x, step):
            return _gate_at(x, marks, span * step, zero)

        def tile(kind, u):
            return jnp.concatenate([buf[r:r + 64, _tile(u)] for r in (kind * 64, 192 + kind * 64)])

        k = [tile(1, t) for t in range(8)]
        v = [tile(2, t) for t in range(8)]
        v_first = jnp.broadcast_to(v[0][:, 0:1], (128, 128))
        k_back = [None] + [pltpu.roll(x, 1, 1) for x in k[1:]]
        v_back = [None] + [jnp.where(first, v_first, pltpu.roll(x, 1, 1)) for x in v[1:]]
        for u in range(8):
            q = tile(0, u).reshape(16, 8, 128)
            logits = []
            for t in range(8):
                if t % 2 == 0:
                    qs = q * paced(jnp.full((8, 128), QK_SCALE, F32), (u + t / 16) / 8)
                lg = jnp.sum(qs * (k[t] if t <= u else k_back[t]).reshape(16, 8, 128), axis=0)
                lg = lg + jnp.where(even, pltpu.roll(lg, 7, 0), pltpu.roll(lg, 1, 0))
                if t > u:
                    lg = jnp.where(first[0:8], MASKED, lg)
                logits.append(lg)
            m = _tree(jnp.maximum, logits)
            p = [jnp.exp2(lg - m) for lg in logits]
            inv = pltpu.reciprocal(_tree(jnp.add, p), full_range=False)
            for part in range(4):
                r = paced(inv, (u + 0.5 + part / 8) / 8)
                o = None
                for t in range(8):
                    x = (v[t] if t <= u else v_back[t]).reshape(16, 8, 128)[_tile(part, 4)]
                    o = (p[t] * r) * x if o is None else o + (p[t] * r) * x
                ot[2 * par + u // 4, _ds(g * 128 + part * 32, 32, 32), _tile(u % 4)] = (
                    o.reshape(32, 128))

    def as_bf16_bits(x):
        return pltpu.bitcast(x.astype(BF16).astype(F32), U32)

    def layer_b(pair):
        zero = _zero_bits(pair)
        qkv_proj(0, 0, first=True)
        marks = []
        qkv_proj(0, 1, marks, first=True)
        window(0, 0, marks, zero, 0.9)

        def mix(g, carry):
            m0, m1 = [], []
            qkv_proj(g, 0, m0)
            window(g - 1, 1, m0, zero, 0.9)
            qkv_proj(g, 1, m1)
            window(g, 0, m1, zero, 0.9)
            return carry
        lax.fori_loop(1, NG, mix, 0)
        marks = []
        out_proj(wobt, 0, marks, 8, 5)
        window(NG - 1, 1, marks, zero, 0.75)

        for n, (kt, t) in enumerate((kt, t) for kt in range(4) for t in range(4)):
            fraction = 0.85 * n / 12 if kt < 3 else 0.8 + (n - 12) * 0.05
            blocks = [jnp.concatenate([_gate_at(ot[b, _tile(k), _tile(t)], marks, fraction, zero)
                                       for k in (kt, kt + 4)]) for b in (2, 3)]
            for i, form in enumerate(_right_forms(*blocks)):
                xn.put(form, i, rows=_rows(kt), cols=_tile(t))

        def b_out(i, carry):
            size = OUT_STRIPS * 128
            rows = _ds(i * size, size, size)
            ys = _strassen(functools.partial(wobt.get, rows=_rows(i, size // 2)),
                           [xn.get(f) for f in range(7)])
            for half in range(2):
                b = 2 + half
                pieces = sorted((p for rh, h, q in ys if h == half for p in _head_halves(q, rh)),
                                key=lambda p: p[0])
                x = xt[b, rows, :] + jnp.concatenate([piece for _, piece in pieces])
                xt[b, rows, :] = x
                pivot = jnp.where(i == 0, x[0:1], stats[b, 2, 0:1])
                s1, s2 = shifted_sums(x, pivot)
                stats[b, 0] = jnp.where(i == 0, 0.0, stats[b, 0]) + s1
                stats[b, 1] = jnp.where(i == 0, 0.0, stats[b, 1]) + s2
                stats[b, 2] = jnp.broadcast_to(pivot, (8, CB))
                words = (as_bf16_bits(xt[half, rows, :]) >> 16) | as_bf16_bits(x)
                for c in range(OUT_STRIPS):
                    for t in range(4):
                        xs_words[i * OUT_STRIPS + c, pl.ds(4 * half + t, 128, stride=8), :] = (
                            words[_tile(c), _tile(t)].T)

            @pl.when(pair == 1)
            def _():
                for c in range(OUT_STRIPS):
                    out_cp(i * OUT_STRIPS + c).start()
            return carry
        lax.fori_loop(0, 8 // OUT_STRIPS, b_out, 0)
        for b in (2, 3):
            put_stats(b, stats[b, 2, 0:1], stats[b, 0], stats[b, 1])

        @pl.when(pair == 1)
        def _():
            for c in range(8):
                out_cp(c).wait()

    def pair_body(pair, carry):
        layer_a(pair)
        layer_b(pair)
        return carry
    lax.fori_loop(0, 2, pair_body, 0)


@jax.jit
def pallas_interleave_layers__grouped_kv_mqa__sliding_local_dilated__prompt_kernel(
    A_x: jax.Array,
    A_wq: jax.Array,
    A_wk: jax.Array,
    A_wv: jax.Array,
    A_wo: jax.Array,
    B_x: jax.Array,
    B_wqkv: jax.Array,
    B_wo: jax.Array,
):
    del B_x
    hbm = pl.BlockSpec(memory_space=pl.ANY)
    vmem = pl.BlockSpec(memory_space=pltpu.VMEM)
    out = pl.pallas_call(
        _kernel,
        in_specs=[hbm, hbm, vmem, vmem, hbm, hbm, hbm],
        out_specs=hbm,
        out_shape=jax.ShapeDtypeStruct((S, D), BF16),
        scratch_shapes=[
            pltpu.VMEM((8, S + 16, 128), BF16),
            pltpu.VMEM((D, D), BF16),
            pltpu.VMEM((D, D), BF16),
            pltpu.VMEM((D, 3 * D), BF16),
            pltpu.VMEM((D, D), BF16),
            pltpu.VMEM((DH, D), U32),
            pltpu.VMEM((7 * CB // 2, D // 2), U32),
            pltpu.VMEM((7 * CB // 2, D // 2), U32),
            pltpu.VMEM((NG * 7 * 96, D // 2), U32),
            pltpu.VMEM((7 * CB // 2, D // 2), U32),
            pltpu.VMEM((NB, D, CB), F32),
            pltpu.VMEM((NB, 3, 8, CB), F32),
            pltpu.VMEM((2 * 7 * CB // 2, CB), U32),
            pltpu.VMEM((NB * D // 2, CB), U32),
            pltpu.VMEM((NB * D + DH * VPU_KEYS // 4, CB), F32),
            pltpu.VMEM((NB, D, CB), F32),
            pltpu.VMEM((4 * S // 2, 128), U32),
            pltpu.VMEM((NB * DH // 2, CB), U32),
            pltpu.VMEM((S, CB), F32),
            pltpu.VMEM((384, 2 * CB), F32),
            pltpu.VMEM((384, 2 * CB), F32),
            pltpu.SemaphoreType.DMA((12,)),
        ],
        compiler_params=pltpu.CompilerParams(vmem_limit_bytes=110 * 1024 * 1024),
        name="interleave_stack",
    )(A_x.reshape(S, D), A_wq, A_wk.T, A_wv.T, A_wo, B_wqkv, B_wo)
    return out.reshape(1, S, D)
```
